```python
import os as _os
_os.environ.setdefault("JAX_PLATFORMS", "cpu")
import jax
import jax.numpy as jnp

def _softmax(x, axis=-1):
    return jax.nn.softmax(x, axis=axis)
def _gelu(x):
    return jax.nn.gelu(x, approximate=True)
def _silu(x):
    return jax.nn.silu(x)
def _sigmoid(x):
    return jax.nn.sigmoid(x)
def _layernorm(x, axis=-1, eps=1e-5):
    m = jnp.mean(x, axis=axis, keepdims=True)
    v = jnp.var(x, axis=axis, keepdims=True)
    return (x - m) / jnp.sqrt(v + eps)
def _scatter_add(tgt, idx, src, axis=0):
    return tgt.at[idx].add(src)
def _segment_sum(src, seg, n):
    return jax.ops.segment_sum(src, seg, n)
class _Rng:
    def __init__(self, key):
        self._k = key
    def _next(self):
        self._k, sub = jax.random.split(self._k)
        return sub
    def normal(self, shape):
        return jax.random.normal(self._next(), shape, dtype=jnp.bfloat16)
    def randint(self, lo, hi, shape):
        return jax.random.randint(self._next(), shape, lo, hi, dtype=jnp.int32)
    def uniform(self, shape, lo=0.0, hi=1.0):
        return jax.random.uniform(self._next(), shape, jnp.bfloat16, lo, hi)
    def permutation(self, n):
        return jax.random.permutation(self._next(), n)


kernel_name = 'sequential_preLN__linear_kernel_hedgehog__geglu_ffn__prompt'

def setup_inputs():
    _rng = _Rng(jax.random.key(int.from_bytes(__import__("os").urandom(4), "little")))
    _w = (lambda a: (lambda t: t.astype(jnp.bfloat16) if jnp.issubdtype(t.dtype, jnp.floating) else t)(jnp.asarray(a)))
    def _A_setup():
        B, S, D, H = 1, 2048, 640, 32
        Dh = D // H
        return {
            "x": _w((lambda *s: _rng.normal(s) * 0.05)(B, S, D)),
            "wqkv": _w((lambda *s: _rng.normal(s) * 0.2)(D, 3 * D)),
            "w_phi": _w((lambda *s: _rng.normal(s) * 0.2)(H, Dh, Dh) * (Dh ** -0.5)),
            "wo": _w((lambda *s: _rng.normal(s) * 0.05)(D, D)),
        }
    _A_in = _A_setup()

    def _B_setup():
        B, S, D, F = 1, 2048, 640, 1536
        return {
            "x": _w((lambda *s: _rng.normal(s) * 0.05)(B, S, D)),
            "w_gate": _w((lambda *s: _rng.normal(s) * 0.05)(D, F)),
            "w_up": _w((lambda *s: _rng.normal(s) * 0.05)(D, F)),
            "w_down": _w((lambda *s: _rng.normal(s) * 0.05)(F, D)),
        }
    _B_in = _B_setup()

    return {
        "A_x": _A_in["x"],
        "A_wqkv": _A_in["wqkv"],
        "A_w_phi": _A_in["w_phi"],
        "A_wo": _A_in["wo"],
        "B_x": _B_in["x"],
        "B_w_gate": _B_in["w_gate"],
        "B_w_up": _B_in["w_up"],
        "B_w_down": _B_in["w_down"],
    }

def reference(A_x, A_wqkv, A_w_phi, A_wo, B_x, B_w_gate, B_w_up, B_w_down):
    def _A_ref(x, wqkv, w_phi, wo):
        B, S, D = x.shape
        H = 32; Dh = D // H
        qkv = (lambda x, *d: x.transpose(*d))((x @ wqkv).reshape(B, S, 3, H, Dh), 2, 0, 3, 1, 4)
        q, k, v = qkv[0], qkv[1], qkv[2]
        pq = jnp.einsum("bhsd,hdf->bhsf", q, w_phi)
        pk = jnp.einsum("bhsd,hdf->bhsf", k, w_phi)
        phi_q = jnp.concatenate([_softmax(pq, axis=-1), _softmax(-pq, axis=-1)], axis=-1)
        phi_k = jnp.concatenate([_softmax(pk, axis=-1), _softmax(-pk, axis=-1)], axis=-1)
        kv = jnp.einsum("bhsf,bhsd->bhfd", phi_k, v)
        z  = jnp.einsum("bhsf->bhf", phi_k)
        num = jnp.einsum("bhqf,bhfd->bhqd", phi_q, kv)
        den = jnp.einsum("bhqf,bhf->bhq", phi_q, z)[..., None] + 1e-6
        o = num / den
        return (lambda x, *d: x.transpose(*d))(o, 0, 2, 1, 3).reshape(B, S, D) @ wo

    def _B_ref(x, w_gate, w_up, w_down):
        return (_gelu(x @ w_gate) * (x @ w_up)) @ w_down

    x = A_x
    h = x + _A_ref(_layernorm(x, axis=-1), A_wqkv, A_w_phi, A_wo)
    h2 = h + _B_ref(_layernorm(h, axis=-1), B_w_gate, B_w_up, B_w_down)
    return h2
```

```python
import functools
import math

import jax
import jax.numpy as jnp
from jax import lax
import jax.experimental.pallas as pl
import jax.experimental.pallas.tpu as pltpu

S, D, H, DH, F = 2048, 640, 32, 20, 1536
NG = 16
GR = 40
PR = 80
VR = 48
NPT = 10
LN_EPS = 1e-5
DEN_EPS = 1e-6
F32 = jnp.float32
BF16 = jnp.bfloat16

NT_DIMS = (((1,), (1,)), ((), ()))
TN_DIMS = (((0,), (0,)), ((), ()))


def _tile_groups(j):
    return (128 * j) // PR, (128 * j + 127) // PR


def _layernorm(x):
    mu = jnp.mean(x, axis=-1, keepdims=True)
    xc = x - mu
    var = jnp.mean(xc * xc, axis=-1, keepdims=True)
    return xc * lax.rsqrt(var + LN_EPS)


def _allred(op, t):
    t = op(t, pltpu.roll(t, 2, 1))
    return op(t, pltpu.roll(t, 4, 1))


def _feature_map(p, n):
    t = p.shape[-1]
    p4 = p.reshape(n, 5, 8, t)
    mx = _allred(jnp.maximum, jnp.max(p4, axis=1))[:, None]
    mn = _allred(jnp.minimum, jnp.min(p4, axis=1))[:, None]
    ep = jnp.exp(p4 - mx)
    en = jnp.exp(mn - p4)
    sp = _allred(jnp.add, jnp.sum(ep, axis=1))[:, None]
    sn = _allred(jnp.add, jnp.sum(en, axis=1))[:, None]
    phi = jnp.concatenate([ep * (1.0 / sp), en * (1.0 / sn)], axis=1)
    return phi.reshape(n * PR, t).astype(BF16)


def _gelu(g):
    c = math.sqrt(2.0 / math.pi)
    return 0.5 * g * (1.0 + jnp.tanh(c * (g + 0.044715 * (g * g * g))))


def _fold_windows():
    wins = []
    for kt in range(5):
        g_lo, g_hi = (128 * kt) // GR, (128 * kt + 127) // GR
        r0 = (g_lo * GR) // 16 * 16
        r1 = -((-(g_hi + 1) * GR) // 16) * 16
        wins.append((r0, r1))
    return wins


def _make_kernel(T, FC):
    NT = S // T
    NC = F // FC
    wins = _fold_windows()

    def kernel(x_hbm, wqkv_hbm, wphi_hbm, wo_hbm, wg_hbm, wu_hbm, wd_hbm,
               o_ref,
               x_v, wphi_v, wk_v, wq_v, wv_v, wo_v, wg_v, wu_v, wd_v,
               wT, xn_s, phiq, kvacc, kvb, kvmask, h_s, hn_s, sems):
        step = pl.program_id(0)

        def cp(k):
            src, dst = [
                (wphi_hbm, wphi_v),
                (x_hbm.at[0:T], x_v.at[0:T]),
                (wqkv_hbm.at[:, D:2 * D], wk_v),
                (wqkv_hbm.at[:, 0:D], wq_v),
                (wqkv_hbm.at[:, 2 * D:3 * D], wv_v),
                (x_hbm.at[T:2 * T], x_v.at[T:2 * T]),
                (x_hbm.at[2 * T:S], x_v.at[2 * T:S]),
                (wo_hbm, wo_v),
                (wg_hbm, wg_v),
                (wu_hbm, wu_v),
                (wd_hbm, wd_v),
            ][k]
            return pltpu.make_async_copy(src, dst, sems.at[k])

        def x_tile(t):
            return x_v[pl.ds(pl.multiple_of(t * T, T), T), :].astype(F32)

        def fold(bdts, w_ref):
            parts = [lax.dot_general(bdts[kt], w_ref[:, 128 * kt:128 * (kt + 1)],
                                     NT_DIMS, preferred_element_type=F32)
                     for kt in range(5)]
            pieces = []
            pos = 0
            for kt in range(5):
                r0, r1 = wins[kt]
                nxt = wins[kt + 1][0] if kt < 4 else r1
                pieces.append(parts[kt][pos - r0:nxt - r0])
                if kt < 4:
                    pieces.append(parts[kt][nxt - r0:] + parts[kt + 1][:r1 - nxt])
                pos = r1
            return jnp.concatenate(pieces, axis=0).astype(BF16)

        @pl.when(step == 0)
        def _prologue():
            for k in range(11):
                cp(k).start()
            kvacc[...] = jnp.zeros(kvacc.shape, F32)
            rel = (lax.broadcasted_iota(jnp.int32, (H, D), 1)
                   - DH * lax.broadcasted_iota(jnp.int32, (H, D), 0))
            e2 = jnp.where(
                lax.broadcasted_iota(jnp.int32, (VR, DH), 0) // 2
                == lax.broadcasted_iota(jnp.int32, (VR, DH), 1), 1.0, 0.0).astype(BF16)
            cp(0).wait()
            m = None
            for d in range(DH):
                sel = jnp.where(rel == d, 1.0, 0.0).astype(BF16)
                t = jnp.dot(wphi_v[d], sel, preferred_element_type=F32)
                m = t if m is None else m + t
            m2 = jnp.dot(e2, m.astype(BF16), preferred_element_type=F32)[0:GR]
            bdts = []
            for kt in range(5):
                r0, r1 = wins[kt]
                nr = r1 - r0
                pat = m2[:, 128 * kt:128 * (kt + 1)]
                rows = []
                r = r0
                while r < r1:
                    o = r % GR
                    n = min(GR - o, r1 - r)
                    rows.append(pat[o:o + n])
                    r += n
                t1 = jnp.concatenate(rows, axis=0)
                row = lax.broadcasted_iota(jnp.int32, (nr, 128), 0) + r0
                col = lax.broadcasted_iota(jnp.int32, (nr, 128), 1) + 128 * kt
                rh = (row // GR) * 2 + row % 2
                bdts.append(jnp.where(col // DH == rh, t1, 0.0).astype(BF16))
            cp(1).wait()
            xn_s[...] = _layernorm(x_tile(0)).astype(BF16)
            cp(2).wait()
            wT[0:D, :] = fold(bdts, wk_v)
            for j in range(5):
                g_lo, _ = _tile_groups(j)
                row = lax.broadcasted_iota(jnp.int32, (3 * VR, 128), 0)
                col = lax.broadcasted_iota(jnp.int32, (3 * VR, 128), 1) + 128 * j
                rg = row // VR
                rr = row - rg * VR
                rhh = jnp.where(rr < GR, rr // DH, (rr - GR) // 4)
                rh = (rg + g_lo) * 2 + rhh
                ch = (col // PR) * 2 + col % 2
                kvmask[j] = jnp.where(rh == ch, 1.0, 0.0)
            cp(3).wait()
            cp(4).wait()
            wT[D:2 * D, :] = fold(bdts, wq_v)
            wT[2 * D:3 * D, :] = wv_v[...].T
            cp(5).wait()

        @pl.when(step == 1)
        def _wait_x():
            cp(6).wait()

        @pl.when(step < NT)
        def _phase1():
            def proj(r0, r1):
                return lax.dot_general(wT[r0:r1, :], xn_s[...], NT_DIMS,
                                       preferred_element_type=F32)
            xn_next = _layernorm(x_tile(jnp.minimum(step + 1, NT - 1))).astype(BF16)
            phik = [None, None]
            phik[0] = _feature_map(proj(0, 320), 8)
            vt3 = proj(2 * D, 3 * D).reshape(NG, GR, T)
            vta = jnp.concatenate([vt3, jnp.ones((NG, 8, T), F32)], axis=1)
            vta = vta.reshape(NG * VR, T).astype(BF16)
            phik[1] = _feature_map(proj(320, 640), 8)
            for c in range(2):
                phiq[step, 640 * c:640 * (c + 1), :] = _feature_map(
                    proj(D + 320 * c, D + 320 * (c + 1)), 8)
            xn_s[...] = xn_next
            for j in range(NPT):
                c, jj = divmod(j, 5)
                g_lo, g_hi = _tile_groups(j)
                nr = (g_hi + 1 - g_lo) * VR
                upd = lax.dot_general(
                    vta[g_lo * VR:(g_hi + 1) * VR, :],
                    phik[c][128 * jj:128 * (jj + 1), :], NT_DIMS,
                    preferred_element_type=F32)
                kvacc[j, 0:nr, :] += upd

        def att_num(ti):
            gnum = [None] * NG
            for j in range(NPT):
                g_lo, g_hi = _tile_groups(j)
                nr = (g_hi + 1 - g_lo) * VR
                part = jnp.dot(kvb[j, 0:nr, :], phiq[ti, 128 * j:128 * (j + 1), :],
                               preferred_element_type=F32)
                for g in range(g_lo, g_hi + 1):
                    blk = part[(g - g_lo) * VR:(g - g_lo + 1) * VR]
                    gnum[g] = blk if gnum[g] is None else gnum[g] + blk
            sub = lax.broadcasted_iota(jnp.int32, (8, T), 0) < 4
            pieces = []
            for g in range(NG):
                rec = 1.0 / (gnum[g][GR:VR] + DEN_EPS)
                rot = pltpu.roll(rec, 4, 0)
                ra = jnp.where(sub, rec, rot)
                rb = jnp.where(sub, rot, rec)
                scale = jnp.concatenate([ra, ra, rec, rb, rb], axis=0)
                pieces.append(gnum[g][0:GR] * scale)
            return jnp.concatenate(pieces, axis=0).astype(BF16).T

        def att_out(ti, o):
            attn = jnp.dot(o, wo_v[...], preferred_element_type=F32)
            h = x_tile(ti) + attn
            h_s[...] = h
            hn_s[...] = _layernorm(h).astype(BF16)

        def gate_up(c):
            sl = slice(c * FC, (c + 1) * FC)
            g = jnp.dot(hn_s[...], wg_v[:, sl], preferred_element_type=F32)
            u = jnp.dot(hn_s[...], wu_v[:, sl], preferred_element_type=F32)
            return (_gelu(g) * u).astype(BF16)

        def down(c, a):
            return jnp.dot(a, wd_v[c * FC:(c + 1) * FC, :],
                           preferred_element_type=F32)

        @pl.when(step == NT)
        def _mid():
            for k in range(7, 11):
                cp(k).wait()
            for j in range(NPT):
                kvb[j] = jnp.where(kvmask[j % 5] > 0.5, kvacc[j], 0.0).astype(BF16)
            att_out(0, att_num(0))

        @pl.when(jnp.logical_and(step >= NT, step < 2 * NT - 1))
        def _phase2():
            tn = step - NT + 1
            a0 = gate_up(0)
            o = att_num(tn)
            acc = h_s[...] + down(0, a0)
            acts = [gate_up(c) for c in range(1, NC)]
            att_out(tn, o)
            for c in range(1, NC):
                acc = acc + down(c, acts[c - 1])
            o_ref[...] = acc.astype(o_ref.dtype)

        @pl.when(step == 2 * NT - 1)
        def _last():
            acc = h_s[...]
            for c in range(NC):
                acc = acc + down(c, gate_up(c))
            o_ref[...] = acc.astype(o_ref.dtype)

    return kernel, NT


def build(T=256, FC=512):
    kernel, NT = _make_kernel(T, FC)

    @jax.jit
    def fn(A_x, A_wqkv, A_w_phi, A_wo, B_x, B_w_gate, B_w_up, B_w_down):
        x = A_x.reshape(S, D)
        wphi = jnp.transpose(A_w_phi, (1, 2, 0))
        any_spec = pl.BlockSpec(memory_space=pl.ANY)
        out = pl.pallas_call(
            kernel,
            grid=(2 * NT,),
            in_specs=[any_spec] * 7,
            out_specs=pl.BlockSpec((T, D), lambda i: (jnp.maximum(i - NT, 0), 0)),
            out_shape=jax.ShapeDtypeStruct((S, D), BF16),
            scratch_shapes=[
                pltpu.VMEM((S, D), BF16),
                pltpu.VMEM((DH, DH, H), BF16),
                pltpu.VMEM((D, D), BF16),
                pltpu.VMEM((D, D), BF16),
                pltpu.VMEM((D, D), BF16),
                pltpu.VMEM((D, D), BF16),
                pltpu.VMEM((D, F), BF16),
                pltpu.VMEM((D, F), BF16),
                pltpu.VMEM((F, D), BF16),
                pltpu.VMEM((3 * D, D), BF16),
                pltpu.VMEM((T, D), BF16),
                pltpu.VMEM((NT, 2 * D, T), BF16),
                pltpu.VMEM((NPT, 3 * VR, 128), F32),
                pltpu.VMEM((NPT, 3 * VR, 128), BF16),
                pltpu.VMEM((5, 3 * VR, 128), F32),
                pltpu.VMEM((T, D), F32),
                pltpu.VMEM((T, D), BF16),
                pltpu.SemaphoreType.DMA((11,)),
            ],
            compiler_params=pltpu.CompilerParams(
                dimension_semantics=("arbitrary",),
                vmem_limit_bytes=100 * 1024 * 1024),
            name="hedgehog_block",
        )(x, A_wqkv, wphi, A_wo, B_w_gate, B_w_up, B_w_down)
        return out.reshape(1, S, D)

    return fn


_impl = build(T=256, FC=512)


@jax.jit
def pallas_sequential_preLN__linear_kernel_hedgehog__geglu_ffn__prompt_kernel(
    A_x: jax.Array,
    A_wqkv: jax.Array,
    A_w_phi: jax.Array,
    A_wo: jax.Array,
    B_x: jax.Array,
    B_w_gate: jax.Array,
    B_w_up: jax.Array,
    B_w_down: jax.Array,
):
    return _impl(A_x, A_wqkv, A_w_phi, A_wo, B_x, B_w_gate, B_w_up, B_w_down)
```

```python
import functools
import math

import jax
import jax.numpy as jnp
from jax import lax
import jax.experimental.pallas as pl
import jax.experimental.pallas.tpu as pltpu

S, D, H, DH, F = 2048, 640, 32, 20, 1536
NG = 16
GR = 40
PR = 80
VR = 48
NPT = 10
LN_EPS = 1e-5
DEN_EPS = 1e-6
F32 = jnp.float32
BF16 = jnp.bfloat16

NT_DIMS = (((1,), (1,)), ((), ()))


def _tile_groups(j):
    return (128 * j) // PR, (128 * j + 127) // PR


def _layernorm(x, anchor=None):
    t = x.shape[0]
    s1 = x[:, 0:128]
    for k in range(1, D // 128):
        s1 = s1 + x[:, 128 * k:128 * (k + 1)]
    if anchor is not None:
        s1 = (s1.reshape(t // 8, 8, 128) + anchor[None]).reshape(t, 128)
    mu = jnp.sum(s1, axis=-1, keepdims=True) * (1.0 / D)
    xc = x - mu
    var = jnp.mean(xc * xc, axis=-1, keepdims=True)
    return xc * lax.rsqrt(var + LN_EPS)


def _allred(op, t):
    t = op(t, pltpu.roll(t, 2, 1))
    return op(t, pltpu.roll(t, 4, 1))


def _feature_map(p, n):
    t = p.shape[-1]
    p4 = p.reshape(n, 5, 8, t)
    mx = _allred(jnp.maximum, jnp.max(p4, axis=1))[:, None]
    mn = _allred(jnp.minimum, jnp.min(p4, axis=1))[:, None]
    ep = jnp.exp(p4 - mx)
    en = jnp.exp(mn - p4)
    sp = _allred(jnp.add, jnp.sum(ep, axis=1))[:, None]
    sn = _allred(jnp.add, jnp.sum(en, axis=1))[:, None]
    phi = jnp.concatenate([ep * (1.0 / sp), en * (1.0 / sn)], axis=1)
    return phi.reshape(n * PR, t).astype(BF16)


def _gelu(g):
    c = math.sqrt(2.0 / math.pi)
    return 0.5 * g * (1.0 + jnp.tanh(c * (g + 0.044715 * (g * g * g))))


def _fold_windows():
    wins = []
    for kt in range(5):
        g_lo, g_hi = (128 * kt) // GR, (128 * kt + 127) // GR
        r0 = (g_lo * GR) // 16 * 16
        r1 = -((-(g_hi + 1) * GR) // 16) * 16
        wins.append((r0, r1))
    return wins


def _make_kernel(T, FC, ANCH, TL, WR, STOP, TQ, MIDS):
    NT = S // T
    NC = F // FC
    TH = T // 2
    wins = _fold_windows()

    def kernel(x_hbm, wqkv_hbm, wphi_hbm, wo_hbm, wg_hbm, wu_hbm, wd_hbm,
               o_hbm,
               x_v, wphi_v, wk_v, wq_v, wv_v, wo_v, wg_v, wu_v, wd_v,
               wT, xn_s, phiq, kvacc, kvb, h_s, hn_s, o_v, zero_s, sems):

        srcs = [
            (wphi_hbm, wphi_v),
            (x_hbm.at[0:TH], x_v.at[0:TH]),
            (wqkv_hbm.at[:, D:2 * D], wk_v),
            (x_hbm.at[TH:T], x_v.at[TH:T]),
            (wqkv_hbm.at[:, 0:D], wq_v),
            (wqkv_hbm.at[:, 2 * D:3 * D], wv_v),
            (x_hbm.at[T:2 * T], x_v.at[T:2 * T]),
            (x_hbm.at[2 * T:S], x_v.at[2 * T:S]),
            (wo_hbm, wo_v),
            (wg_hbm, wg_v),
            (wu_hbm, wu_v),
            (wd_hbm, wd_v),
        ]

        sem_of = [0, 0, 1, 2, 2, 3, 3, 4, 5, 5, 5, 5]

        def cp(k):
            return pltpu.make_async_copy(srcs[k][0], srcs[k][1], sems.at[sem_of[k]])

        def x_rows(r0, n):
            return x_v[pl.ds(pl.multiple_of(r0, 16), n), :].astype(F32)

        def fold(bdts, w_ref):
            parts = [lax.dot_general(bdts[kt], w_ref[:, 128 * kt:128 * (kt + 1)],
                                     NT_DIMS, preferred_element_type=F32)
                     for kt in range(5)]
            pieces = []
            pos = 0
            for kt in range(5):
                r0, r1 = wins[kt]
                nxt = wins[kt + 1][0] if kt < 4 else r1
                pieces.append(parts[kt][pos - r0:nxt - r0])
                if kt < 4:
                    pieces.append(parts[kt][nxt - r0:] + parts[kt + 1][:r1 - nxt])
                pos = r1
            return jnp.concatenate(pieces, axis=0).astype(BF16)

        def proj(r0, r1, xn):
            return lax.dot_general(wT[r0:r1, :], xn, NT_DIMS,
                                   preferred_element_type=F32)

        def kmap(c, xn):
            return _feature_map(proj(320 * c, 320 * (c + 1), xn), 8)

        def p1_tail(t, cur, phik, zero):
            for c in range(2):
                phiq[t, 640 * c:640 * (c + 1), :] = _feature_map(
                    proj(D + 320 * c, D + 320 * (c + 1), xn_s[cur]), 8)
            anchors = []
            vta = []
            for c in range(2):
                vt = proj(2 * D + 320 * c, 2 * D + 320 * (c + 1), xn_s[cur])
                for n in range(T // 128):
                    for r in ANCH:
                        sl = vt[r:r + 8, 128 * n:128 * (n + 1)]
                        anchors.append(pltpu.bitcast(
                            pltpu.bitcast(sl, jnp.int32) & zero, F32))
                va = jnp.concatenate([vt.reshape(8, GR, T),
                                      jnp.ones((8, 8, T), F32)], axis=1)
                vta.append(va.reshape(8 * VR, T).astype(BF16))
            base = jnp.minimum(t + 1, NT - 1) * T
            lnc = T // len(anchors)
            for i, an in enumerate(anchors):
                r = i * lnc
                xn_s[1 - cur, r:r + lnc, :] = _layernorm(
                    x_rows(base + r, lnc), an).astype(BF16)
            for j in range(NPT):
                c, jj = divmod(j, 5)
                g_lo, g_hi = _tile_groups(jj)
                nr = (g_hi + 1 - g_lo) * VR
                upd = lax.dot_general(
                    vta[c][g_lo * VR:(g_hi + 1) * VR, :],
                    phik[c][128 * jj:128 * (jj + 1), :], NT_DIMS,
                    preferred_element_type=F32)
                kvacc[j, 0:nr, :] += upd

        for k in range(len(srcs) if STOP > 1 else 8):
            cp(k).start()
        zero_s[0] = 0
        kvacc[...] = jnp.zeros(kvacc.shape, F32)
        rel = (lax.broadcasted_iota(jnp.int32, (H, D), 1)
               - DH * lax.broadcasted_iota(jnp.int32, (H, D), 0))
        e2 = jnp.where(
            lax.broadcasted_iota(jnp.int32, (VR, DH), 0) >> 1
            == lax.broadcasted_iota(jnp.int32, (VR, DH), 1), 1.0, 0.0).astype(BF16)
        lane8 = lax.broadcasted_iota(jnp.int32, (8, 128), 1)
        sub8 = lax.broadcasted_iota(jnp.int32, (8, 128), 0)
        cp(0).wait()
        cp(1).wait()
        m = None
        for d in range(DH):
            sel = jnp.where(rel == d, 1.0, 0.0).astype(BF16)
            t = jnp.dot(wphi_v[d], sel, preferred_element_type=F32)
            m = t if m is None else m + t
        m2 = jnp.dot(e2, m.astype(BF16), preferred_element_type=F32)[0:GR]
        relp = lane8 - DH * (sub8 & 1)
        bdts = []
        for kt in range(5):
            r0, r1 = wins[kt]
            pat = m2[:, 128 * kt:128 * (kt + 1)].reshape(5, 8, 128)
            rows = []
            r = r0
            while r < r1:
                g, o = divmod(r, GR)
                n = min(GR - o, r1 - r)
                c0 = GR * g - 128 * kt
                msk = jnp.logical_and(relp >= c0, relp < c0 + DH)
                rows.append(jnp.where(msk[None], pat[o // 8:(o + n) // 8], 0.0))
                r += n
            bdts.append(jnp.concatenate(rows, axis=0)
                        .reshape(r1 - r0, 128).astype(BF16))
        xn_s[0, 0:TH, :] = _layernorm(x_rows(0, TH)).astype(BF16)
        cp(2).wait()
        wT[0:D, :] = fold(bdts, wk_v)
        pka = [kmap(c, xn_s[0, 0:TH, :]) for c in range(2)]
        cp(3).wait()
        cp(4).wait()
        xn_s[0, TH:T, :] = _layernorm(x_rows(TH, TH)).astype(BF16)
        wT[D:2 * D, :] = fold(bdts, wq_v)
        pkb = [kmap(c, xn_s[0, TH:T, :]) for c in range(2)]
        cp(5).wait()
        cp(6).wait()
        wT[2 * D:3 * D, :] = wv_v[...].T
        p1_tail(0, 0,
                [jnp.concatenate([pka[c], pkb[c]], axis=1) for c in range(2)],
                zero_s[0])
        cp(7).wait()
        if STOP == 0:
            return

        def p1_body(t, carry):
            cur = t % 2
            phik = [kmap(c, xn_s[cur]) for c in range(2)]
            p1_tail(t, cur, phik, zero_s[0])
            return carry

        lax.fori_loop(1, NT, p1_body, 0)
        if STOP == 1:
            return

        def att_num(ti):
            gnum = [None] * NG
            for j in range(NPT):
                g_lo, g_hi = _tile_groups(j)
                nr = (g_hi + 1 - g_lo) * VR
                part = jnp.dot(kvb[j, 0:nr, :], phiq[ti, 128 * j:128 * (j + 1), :],
                               preferred_element_type=F32)
                for g in range(g_lo, g_hi + 1):
                    blk = part[(g - g_lo) * VR:(g - g_lo + 1) * VR]
                    gnum[g] = blk if gnum[g] is None else gnum[g] + blk
            sub = lax.broadcasted_iota(jnp.int32, (8, T), 0) < 4
            pieces = []
            for g in range(NG):
                rec = 1.0 / (gnum[g][GR:VR] + DEN_EPS)
                rot = pltpu.roll(rec, 4, 0)
                ra = jnp.where(sub, rec, rot)
                rb = jnp.where(sub, rot, rec)
                scale = jnp.concatenate([ra, ra, rec, rb, rb], axis=0)
                pieces.append(gnum[g][0:GR] * scale)
            return jnp.concatenate(pieces, axis=0).astype(BF16).T

        def att_out(ti, o, splits):
            r = 0
            for n in splits:
                attn = jnp.dot(o[r:r + n], wo_v[...], preferred_element_type=F32)
                h = x_rows(ti * T + r, n) + attn
                h_s[r:r + n, :] = h
                hn_s[r:r + n, :] = _layernorm(h).astype(BF16)
                r += n

        def gate_up(c, rows):
            sl = slice(c * FC, (c + 1) * FC)
            g = jnp.dot(hn_s[rows, :], wg_v[:, sl], preferred_element_type=F32)
            u = jnp.dot(hn_s[rows, :], wu_v[:, sl], preferred_element_type=F32)
            return (_gelu(g) * u).astype(BF16)

        def down(c, a):
            return jnp.dot(a, wd_v[c * FC:(c + 1) * FC, :],
                           preferred_element_type=F32)

        def out_cp(r0, n, sem):
            rows = pl.ds(pl.multiple_of(r0, 16), n)
            return pltpu.make_async_copy(o_v.at[rows], o_hbm.at[rows], sems.at[0])

        for k in range(8, 12):
            cp(k).wait()
        odd = lane8 & 1
        hi = (sub8 >= 4).astype(jnp.int32)
        for j in range(NPT):
            g_lo, g_hi = _tile_groups(j)
            for g in range(g_lo, g_hi + 1):
                c0 = PR * g - 128 * j
                rng = jnp.logical_and(lane8 >= c0, lane8 < c0 + PR)
                me = jnp.logical_and(rng, odd == 0)
                mo = jnp.logical_and(rng, odd == 1)
                mm = jnp.logical_and(rng, odd == hi)
                r0 = (g - g_lo) * VR
                blk = kvacc[j, r0:r0 + VR, :]
                kvb[j, r0:r0 + VR, :] = jnp.concatenate(
                    [jnp.where(mk, blk[8 * i:8 * (i + 1)], 0.0)
                     for i, mk in enumerate((me, me, mm, mo, mo, mm))],
                    axis=0).astype(BF16)
        att_out(0, att_num(0), MIDS)
        if STOP == 2:
            return

        def p2_body(t, carry):
            allr = slice(0, T)
            a0 = gate_up(0, allr)
            o = att_num(t + 1)
            acc = h_s[...] + down(0, a0)
            acts = [gate_up(c, allr) for c in range(1, NC)]
            att_out(t + 1, o, [WR] * (T // WR))
            for c in range(1, NC):
                acc = acc + down(c, acts[c - 1])
            o_v[pl.ds(pl.multiple_of(t * T, T), T), :] = acc.astype(BF16)
            out_cp(t * T, T, t).start()
            return carry

        lax.fori_loop(0, NT - 1, p2_body, 0)

        NQ = TL // TQ

        def last_body(i, carry):
            rows = pl.ds(pl.multiple_of(i * TL, TL), TL)
            acc = h_s[rows, :]
            for c in range(NC - 1):
                acc = acc + down(c, gate_up(c, rows))
            a = gate_up(NC - 1, rows)
            for q in range(NQ):
                res = acc[q * TQ:(q + 1) * TQ] + down(NC - 1, a[q * TQ:(q + 1) * TQ])
                r0 = (NT - 1) * T + i * TL + q * TQ
                o_v[pl.ds(pl.multiple_of(r0, TQ), TQ), :] = res.astype(BF16)
                out_cp(r0, TQ, NT - 1 + i * NQ + q).start()
            return carry

        lax.fori_loop(0, T // TL, last_body, 0)
        pltpu.make_async_copy(o_v, o_hbm, sems.at[0]).wait()

    return kernel, NT


def build(T=512, FC=512, ANCH=(0, 80, 160, 240), TL=256, WR=128, STOP=9, TQ=64,
          MIDS=(128, 128, 128, 64, 64)):
    kernel, NT = _make_kernel(T, FC, ANCH, TL, WR, STOP, TQ, MIDS)

    @jax.jit
    def fn(A_x, A_wqkv, A_w_phi, A_wo, B_x, B_w_gate, B_w_up, B_w_down):
        x = A_x.reshape(S, D)
        wphi = jnp.transpose(A_w_phi, (1, 2, 0))
        any_spec = pl.BlockSpec(memory_space=pl.ANY)
        out = pl.pallas_call(
            kernel,
            in_specs=[any_spec] * 7,
            out_specs=any_spec,
            out_shape=jax.ShapeDtypeStruct((S, D), BF16),
            scratch_shapes=[
                pltpu.VMEM((S, D), BF16),
                pltpu.VMEM((DH, DH, H), BF16),
                pltpu.VMEM((D, D), BF16),
                pltpu.VMEM((D, D), BF16),
                pltpu.VMEM((D, D), BF16),
                pltpu.VMEM((D, D), BF16),
                pltpu.VMEM((D, F), BF16),
                pltpu.VMEM((D, F), BF16),
                pltpu.VMEM((F, D), BF16),
                pltpu.VMEM((3 * D, D), BF16),
                pltpu.VMEM((2, T, D), BF16),
                pltpu.VMEM((NT, 2 * D, T), BF16),
                pltpu.VMEM((NPT, 3 * VR, 128), F32),
                pltpu.VMEM((NPT, 3 * VR, 128), BF16),
                pltpu.VMEM((T, D), F32),
                pltpu.VMEM((T, D), BF16),
                pltpu.VMEM((S, D), BF16),
                pltpu.SMEM((1,), jnp.int32),
                pltpu.SemaphoreType.DMA((6,)),
            ],
            compiler_params=pltpu.CompilerParams(
                vmem_limit_bytes=100 * 1024 * 1024),
            name="hedgehog_block",
        )(x, A_wqkv, wphi, A_wo, B_w_gate, B_w_up, B_w_down)
        return out.reshape(1, S, D)

    return fn


_impl = build(T=512, TQ=64, MIDS=(128, 128, 128, 128))


@jax.jit
def pallas_sequential_preLN__linear_kernel_hedgehog__geglu_ffn__prompt_kernel(
    A_x: jax.Array,
    A_wqkv: jax.Array,
    A_w_phi: jax.Array,
    A_wo: jax.Array,
    B_x: jax.Array,
    B_w_gate: jax.Array,
    B_w_up: jax.Array,
    B_w_down: jax.Array,
):
    return _impl(A_x, A_wqkv, A_w_phi, A_wo, B_x, B_w_gate, B_w_up, B_w_down)
```

```python
import functools
import math

import jax
import jax.numpy as jnp
from jax import lax
import jax.experimental.pallas as pl
import jax.experimental.pallas.tpu as pltpu

S, D, H, DH, F = 2048, 640, 32, 20, 1536
NG = 16
GR = 40
PR = 80
VR = 48
DHALF = D // 2
KH = 256
FH = F // 2
HB = 128
PG = 16
LN_EPS = 1e-5
DEN_EPS = 1e-6
LOG2E = math.log2(math.e)
F32 = jnp.float32
BF16 = jnp.bfloat16
U32 = jnp.uint32


def _dot(a, b):
    return jnp.dot(a, b, preferred_element_type=F32)


def _dot_nt(a, b):
    return lax.dot_general(a, b, (((1,), (1,)), ((), ())),
                           preferred_element_type=F32)


def _pk(v):
    return pltpu.bitcast(v.astype(BF16), U32)


def _upk(w):
    return pltpu.bitcast(w, BF16)


def _ipk(ev, od):
    return pltpu.pack_elementwise([ev, od], packed_dtype=BF16)


def _iupk(w):
    return jnp.concatenate(
        [pltpu.unpack_elementwise(w, index=i, packed_dtype=BF16, unpacked_dtype=F32)
         for i in range(2)], axis=0)


def _ipk2(v):
    n = v.shape[0] // 2
    return _ipk(v[:n], v[n:])


def _hs(a, b):
    assert a % 16 == 0 and b % 16 == 0
    return slice(a // 2, b // 2)


def _layernorm(x, anchor=None):
    t = x.shape[0]
    s1 = x[:, 0:128]
    for k in range(1, D // 128):
        s1 = s1 + x[:, 128 * k:128 * (k + 1)]
    if anchor is not None:
        s1 = (s1.reshape(t // 8, 8, 128) + anchor[None]).reshape(t, 128)
    mu = jnp.sum(s1, axis=-1, keepdims=True) * (1.0 / D)
    xc = x - mu
    var = jnp.mean(xc * xc, axis=-1, keepdims=True)
    return xc * lax.rsqrt(var + LN_EPS)


def _allred(op, t):
    t = op(t, pltpu.roll(t, 2, 1))
    return op(t, pltpu.roll(t, 4, 1))


def _recip(s):
    r = pl.reciprocal(s, approx=True)
    return r * (2.0 - s * r)


def _feature_map(p):
    n, t = p.shape[0] // GR, p.shape[1]
    p4 = p.reshape(n, 5, 8, t)
    mx = _allred(jnp.maximum, jnp.max(p4, axis=1))[:, None]
    mn = _allred(jnp.minimum, jnp.min(p4, axis=1))[:, None]
    ep = jnp.exp2(p4 - mx)
    en = jnp.exp2(mn - p4)
    sp = _allred(jnp.add, jnp.sum(ep, axis=1))[:, None]
    sn = _allred(jnp.add, jnp.sum(en, axis=1))[:, None]
    return _ipk(ep * _recip(sp), en * _recip(sn)).reshape(n * GR, t)


def _augment_v(vt):
    n, t = vt.shape[0] // GR, vt.shape[1]
    va = jnp.concatenate([vt.reshape(n, GR, t), jnp.ones((n, 8, t), F32)], axis=1)
    return va.reshape(n * VR, t)


def _gelu(g):
    c = math.sqrt(2.0 / math.pi)
    return 0.5 * g * (1.0 + jnp.tanh(c * (g + 0.044715 * (g * g * g))))


def _lhs_sums(a11, a12, a21, a22):
    return [a11 + a22, a21 + a22, a11 + a12, a21 - a11, a12 - a22]


def _rhs_sums(b11, b12, b21, b22):
    return [b11 + b22, b12 - b22, b21 - b11, b11 + b12, b21 + b22]


def _lhs_ops(s, a11, a22):
    return [s[0], s[1], a11, a22, s[2], s[3], s[4]]


def _rhs_ops(s, b11, b22):
    return [s[0], b11, s[1], s[2], b22, s[3], s[4]]


def _strassen(dot, lhs, rhs, c11, c12, c21, c22, post=None):
    ev = lambda c: c() if callable(c) else c
    mm = lambda i: dot(ev(lhs[i]), ev(rhs[i]))
    fin = post if post is not None else (lambda _, c: c)
    m2 = mm(2)
    m4 = mm(4)
    c12 = fin(1, m2 + m4 + ev(c12))
    m3 = mm(3)
    m1 = mm(1)
    c21 = fin(2, m3 + m1 + ev(c21))
    m0 = mm(0)
    c11 = fin(0, m3 - m4 + m0 + mm(6) + ev(c11))
    c22 = fin(3, m2 - m1 + m0 + mm(5) + ev(c22))
    return c11, c12, c21, c22


def _strassen_steps(dot, lhs, rhs, rest, post, out):
    mm = lambda i: dot(lhs[i](), rhs[i]())
    m2 = mm(2)
    yield
    m4 = mm(4)
    yield
    out[1] = post(1, m2 + m4 + rest[1]())
    yield
    m3 = mm(3)
    yield
    m1 = mm(1)
    yield
    out[2] = post(2, m3 + m1 + rest[2]())
    yield
    m0 = mm(0)
    yield
    c11 = m3 - m4 + m0 + mm(6)
    yield
    out[0] = post(0, c11 + rest[0]())
    yield
    c22 = m2 - m1 + m0 + mm(5)
    yield
    out[3] = post(3, c22 + rest[3]())
    yield


def _chain(gens):
    for g in gens:
        yield from g


def _split_rows(a):
    n, c = a.shape
    a4 = a.reshape(n // (2 * PG), 2, PG, c)
    return a4[:, 0].reshape(n // 2, c), a4[:, 1].reshape(n // 2, c)


def _merge_rows(top, bot):
    n, c = top.shape
    both = jnp.stack([top.reshape(n // PG, PG, c), bot.reshape(n // PG, PG, c)],
                     axis=1)
    return both.reshape(2 * n, c)


def _fold_windows():
    wins = []
    for kt in range(5):
        g_lo, g_hi = (128 * kt) // GR, (128 * kt + 127) // GR
        r0 = (g_lo * GR) // 16 * 16
        r1 = -((-(g_hi + 1) * GR) // 16) * 16
        wins.append((r0, r1))
    return wins


def _make_kernel(T, TQ, QF, KF, NW, JC, PW, PST, LW, AW, NB, VOFF, MORD):
    NT = S // T
    TH = T // 2
    wins = _fold_windows()
    npair = FH // NW

    def kernel(x_hbm, wqkv_hbm, wphi_hbm, wo_hbm, wg_hbm, wu_hbm, wd_hbm,
               o_hbm,
               x_v, wphi_v, wk_v, wq_v, wv_v, wo_v, wg_v, wu_v, wd_v,
               wT, wS, xn0, xs, x5, phiq, kvacc, kvb, sg, su, sd, o_v, phik_s,
               zero_s, sems):

        srcs = [
            (wphi_hbm, wphi_v),
            (wqkv_hbm.at[:, D:D + 128 * KF], wk_v.at[:, 0:128 * KF]),
            (x_hbm.at[0:TH], x_v.at[0:TH]),
            (wqkv_hbm.at[:, D + 128 * KF:2 * D], wk_v.at[:, 128 * KF:D]),
            (x_hbm.at[TH:T], x_v.at[TH:T]),
            (wqkv_hbm.at[:, 0:D], wq_v),
            (wqkv_hbm.at[:, 2 * D:3 * D], wv_v),
            (x_hbm.at[T:2 * T], x_v.at[T:2 * T]),
            (x_hbm.at[2 * T:S], x_v.at[2 * T:S]),
            (wo_hbm, wo_v),
            (wg_hbm, wg_v),
            (wu_hbm, wu_v),
            (wd_hbm, wd_v),
        ]
        sem_of = [0, 1, 2, 2, 3, 3, 4, 4, 5, 6, 6, 6, 6]

        def cp(k):
            return pltpu.make_async_copy(srcs[k][0], srcs[k][1], sems.at[sem_of[k]])

        def x_rows(r0, n):
            return x_v[pl.ds(pl.multiple_of(r0, 16), n), :].astype(F32)

        def fold_part(kt, bdts, w_ref):
            return _dot_nt(bdts[kt], w_ref[:, 128 * kt:128 * (kt + 1)])

        def fold_store(base, parts, kts):
            for kt in kts:
                r0, r1 = wins[kt]
                pos = r0
                pieces = []
                if kt > 0:
                    p0, p1 = wins[kt - 1]
                    pieces.append(parts[kt - 1][r0 - p0:] + parts[kt][:p1 - r0])
                    pos = p1
                nxt = wins[kt + 1][0] if kt < 4 else r1
                pieces.append(parts[kt][pos - r0:nxt - r0])
                wT[_hs(base + r0, base + nxt), :] = _pk(
                    jnp.concatenate(pieces, axis=0) * LOG2E)

        pace = []

        def note(p):
            tiles = [p[r:r + 8, 128 * n:128 * (n + 1)]
                     for n in range(p.shape[1] // 128)
                     for r in range(0, p.shape[0], PST)]
            pace.append(tiles)
            return p

        def anchors(weights, count):
            pool = []
            for tiles, w in zip(pace[-len(weights):], weights):
                for tl in tiles:
                    pool += [tl] * w
            zero = zero_s[0]
            return [pltpu.bitcast(pool[i * len(pool) // count], U32) & zero
                    for i in range(count)]

        def paced(bits, an):
            rr, cc = bits.shape
            an = jnp.concatenate([an] * (cc // 128), axis=1)
            return (bits.reshape(rr // 8, 8, cc) | an[None]).reshape(rr, cc)

        def block_sums(specs, sums, weights):
            jobs = [(w, dst, rb, k2, n2, r, c)
                    for w, dst, rb, k2, n2 in specs
                    for r in range(0, k2, 16) for c in range(0, n2, JC)]
            for an, (w, dst, rb, k2, n2, r, c) in zip(
                    anchors(weights, len(jobs)), jobs):
                lo, hi = slice(c, c + JC), slice(n2 + c, n2 + c + JC)
                if w.dtype == U32:
                    get = lambda r0, cols: w[_hs(r0, r0 + 16), cols]
                else:
                    get = lambda r0, cols: pltpu.bitcast(w[r0:r0 + 16, cols], U32)
                top, bot = rb + r, rb + k2 + r
                d11, d22 = paced(get(top, lo), an), paced(get(bot, hi), an)
                vals = sums(_iupk(d11), _iupk(get(top, hi)),
                            _iupk(get(bot, lo)), _iupk(d22))
                for j, v in enumerate(vals):
                    dst[j, _hs(r, r + 16), lo] = _ipk2(v)
                if w.dtype != U32:
                    dst[5, _hs(r, r + 16), lo] = d11
                    dst[6, _hs(r, r + 16), lo] = d22

        def ln_pair(r0, anchor=None):
            bits = pltpu.bitcast(
                x_v[pl.ds(pl.multiple_of(r0, 2 * PG), 2 * PG), :], U32)
            xn = _layernorm(jnp.concatenate(
                [_iupk(bits[:PG // 2]), _iupk(bits[PG // 2:])], axis=0), anchor)
            return xn[:PG], xn[PG:]

        def ln_next(t, weights):
            n = T // (2 * PG)
            for i, an in enumerate(anchors(weights, n)):
                lo, hi = ln_pair(t * T + 2 * PG * i, pltpu.bitcast(an, F32))
                b11, b12 = lo[:, 0:KH], hi[:, 0:KH]
                b21, b22 = lo[:, KH:2 * KH], hi[:, KH:2 * KH]
                rows = _hs(PG * i, PG * (i + 1))
                ops = _rhs_ops(_rhs_sums(b11, b12, b21, b22), b11, b22)
                for j, v in enumerate(ops):
                    xs[j, rows, :] = _ipk2(v)
                x5[rows, :] = _ipk2(jnp.concatenate(
                    [lo[:, 2 * KH:], hi[:, 2 * KH:]], axis=1))

        def proj0(r0, xn):
            return note(_dot_nt(_upk(wT[_hs(r0, r0 + DHALF), :]), xn))

        def proj_steps(m, n, post, out):
            top = _hs(m * D, m * D + DHALF)
            bot = _hs(m * D + DHALF, (m + 1) * D)
            tok = _hs(NB * n, NB * (n + 1))
            lhs = _lhs_ops([lambda j=j: _upk(wS[m, j]) for j in range(5)],
                           lambda: _upk(wT[top, 0:KH]),
                           lambda: _upk(wT[bot, KH:2 * KH]))
            rhs = [lambda j=j: _upk(xs[j, tok, :]) for j in range(7)]
            rest = [lambda r=r, c=c: _dot_nt(_upk(wT[r, 2 * KH:D]),
                                             _upk(x5[tok, 128 * c:128 * (c + 1)]))
                    for r in (top, bot) for c in range(2)]
            return _strassen_steps(lambda a, b: note(_dot_nt(a, b)), lhs, rhs, rest,
                                   post, out)

        def kv_update(phik, vta, last):
            if last:
                row = lax.broadcasted_iota(jnp.int32, (VR, PR), 0)
                odd = (lax.broadcasted_iota(jnp.int32, (VR, PR), 1) >> 1) & 1
                second = jnp.logical_or(
                    jnp.logical_and(row >= DH, row < GR), row >= GR + 4)
                keep = odd == second.astype(jnp.int32)
            for g in range(NG):
                c, gg = divmod(g, 8)
                upd = _dot_nt(vta[c][gg * VR:(gg + 1) * VR, :].astype(BF16),
                              _upk(phik[c][gg * GR:(gg + 1) * GR, :]))
                if last:
                    kvb[g] = _pk(jnp.where(keep, kvacc[g] + upd, 0.0))
                else:
                    kvacc[g] += upd

        for k in range(len(srcs)):
            cp(k).start()
        zero_s[0] = jnp.uint32(0)
        kvacc[...] = jnp.zeros(kvacc.shape, F32)
        rel = (lax.broadcasted_iota(jnp.int32, (H, D), 1)
               - DH * lax.broadcasted_iota(jnp.int32, (H, D), 0))
        e2 = jnp.where(
            lax.broadcasted_iota(jnp.int32, (VR, DH), 0) >> 1
            == lax.broadcasted_iota(jnp.int32, (VR, DH), 1), 1.0, 0.0).astype(BF16)
        lane8 = lax.broadcasted_iota(jnp.int32, (8, 128), 1)
        sub8 = lax.broadcasted_iota(jnp.int32, (8, 128), 0)
        cp(0).wait()
        m = None
        for d in range(DH):
            sel = jnp.where(rel == d, 1.0, 0.0).astype(BF16)
            t = _dot(wphi_v[d], sel)
            m = t if m is None else m + t
        m2 = _dot(e2, m.astype(BF16))[0:GR]
        relp = lane8 - DH * (sub8 & 1)
        bdts = []
        for kt in range(5):
            r0, r1 = wins[kt]
            pat = m2[:, 128 * kt:128 * (kt + 1)].reshape(5, 8, 128)
            rows = []
            r = r0
            while r < r1:
                g, o = divmod(r, GR)
                n = min(GR - o, r1 - r)
                c0 = GR * g - 128 * kt
                msk = jnp.logical_and(relp >= c0, relp < c0 + DH)
                rows.append(jnp.where(msk[None], pat[o // 8:(o + n) // 8], 0.0))
                r += n
            bdts.append(jnp.concatenate(rows, axis=0)
                        .reshape(r1 - r0, 128).astype(BF16))

        def ln0(b):
            for i in range(TH // (2 * PG)):
                lo, hi = ln_pair(b * TH + 2 * PG * i)
                r = TH // 2 * b + PG * i
                xn0[_hs(r, r + PG), :] = _ipk2(lo)
                xn0[_hs(TH + r, TH + r + PG), :] = _ipk2(hi)

        def xn0_half(b):
            q = TH // 2
            return _upk(jnp.concatenate(
                [xn0[_hs(q * b, q * (b + 1)), :],
                 xn0[_hs(TH + q * b, TH + q * (b + 1)), :]], axis=0))

        cp(1).wait()
        parts = [fold_part(kt, bdts, wk_v) for kt in range(KF)]
        fold_store(0, parts, range(KF))
        cp(2).wait()
        cp(3).wait()
        ln0(0)
        parts += [fold_part(kt, bdts, wk_v) for kt in range(KF, 5)]
        fold_store(0, parts, range(KF, 5))
        pka = [_feature_map(proj0(DHALF * c, xn0_half(0))) for c in range(2)]
        cp(4).wait()
        cp(5).wait()
        ln0(1)
        qparts = [fold_part(kt, bdts, wq_v) for kt in range(QF)]
        fold_store(D, qparts, range(QF))
        pkb = [_feature_map(proj0(DHALF * c, xn0_half(1))) for c in range(2)]
        qparts += [fold_part(kt, bdts, wq_v) for kt in range(QF, 5)]
        fold_store(D, qparts, range(QF, 5))
        cp(6).wait()
        cp(7).wait()
        wT[_hs(2 * D, 3 * D), :] = _pk(wv_v[...].T)
        for c in range(2):
            phiq[0, _hs(D * c, D * (c + 1)), :] = _feature_map(
                proj0(D + DHALF * c, _upk(xn0[...])))
        vta = [_augment_v(proj0(2 * D + DHALF * c, _upk(xn0[...]))) for c in range(2)]
        ln_next(1, (1, 1))
        block_sums([(wT, wS.at[i], i * D, DHALF, KH) for i in range(3)],
                   _lhs_sums, AW)
        q4 = TH // 2
        kv_update([jnp.concatenate([pka[c][:, :q4], pkb[c][:, :q4],
                                    pka[c][:, q4:], pkb[c][:, q4:]], axis=1)
                   for c in range(2)], vta, False)
        cp(8).wait()

        def p1_body(t, carry):
            last = isinstance(t, int)
            nb = TH // NB
            outs = [[[None] * 4 for _ in range(nb)] for _ in range(3)]
            fm = lambda i, c: _feature_map(c)
            main = _chain([proj_steps(m, n, fm, outs[m][n]) for m, n in MORD])
            side = _chain([proj_steps(2, n, lambda i, c: _augment_v(c), outs[2][n])
                           for n in range(nb)])
            i = 0
            for _ in main:
                i += 1
                if i >= VOFF and i % 2 == 0:
                    next(side, None)
            for _ in side:
                pass

            def gather(m, r):
                return jnp.concatenate([outs[m][n][2 * r + hi] for hi in range(2)
                                        for n in range(nb)], axis=1)

            for r in range(2):
                phiq[t, _hs(D * r, D * (r + 1)), :] = gather(1, r)
            npace = 21 * nb
            if last:
                block_sums([(wg_v, sg, 0, KH, FH), (wu_v, su, 0, KH, FH),
                            (wd_v, sd, 0, FH, KH)], _rhs_sums, (1,) * npace)
            else:
                ln_next(t + 1, (1,) * npace)
            for r in range(2):
                phik_s[r] = gather(0, r)
            kv_update([phik_s.at[r] for r in range(2)],
                      [gather(2, r) for r in range(2)], last)
            return carry

        lax.fori_loop(1, NT - 1, p1_body, 0)
        for k in range(9, 13):
            cp(k).wait()
        p1_body(NT - 1, 0)

        def att_num(ti, b):
            n = 256

            def phi(g):
                rows = _hs(PR * g, PR * (g + 1))
                return _upk(jnp.concatenate(
                    [phiq[ti, rows, c0:c0 + 128] for c0 in (128 * b, TH + 128 * b)],
                    axis=1))

            gnum = [_dot(_upk(kvb[g]), phi(g)) for g in range(NG)]
            sub = lax.broadcasted_iota(jnp.int32, (8, n), 0) < 4
            pieces = []
            for g in range(NG):
                rec = 1.0 / (gnum[g][GR:VR] + DEN_EPS)
                rot = pltpu.roll(rec, 4, 0)
                ra = jnp.where(sub, rec, rot)
                rb = jnp.where(sub, rot, rec)
                scale = jnp.concatenate([ra, ra, rec, rb, rb], axis=0)
                pieces.append(gnum[g][0:GR] * scale)
            o = jnp.concatenate(pieces, axis=0).astype(BF16).T
            return _merge_rows(o[:n // 2], o[n // 2:])

        def att_out(ti, r, o):
            h = x_rows(ti * T + r, o.shape[0]) + _dot(o, wo_v[...])
            return h, _layernorm(h)

        def out_cp(r0, n):
            rows = pl.ds(pl.multiple_of(r0, 16), n)
            return pltpu.make_async_copy(o_v.at[rows], o_hbm.at[rows], sems.at[0])

        def bf16_lhs(a11, a12, a21, a22):
            return [v.astype(BF16)
                    for v in _lhs_ops(_lhs_sums(a11, a12, a21, a22), a11, a22)]

        def ffn(base, chunks, tq):
            ht, hb = _split_rows(jnp.concatenate([c[0] for c in chunks], axis=0))
            nt_, nb = _split_rows(jnp.concatenate([c[1] for c in chunks], axis=0))
            lhs = bf16_lhs(nt_[:, 0:KH], nt_[:, KH:2 * KH],
                           nb[:, 0:KH], nb[:, KH:2 * KH])
            a5 = [nt_[:, 2 * KH:].astype(BF16), nb[:, 2 * KH:].astype(BF16)]
            cs = (ht[:, 0:KH], ht[:, KH:2 * KH], hb[:, 0:KH], hb[:, KH:2 * KH])
            c5 = jnp.concatenate([ht[:, 2 * KH:], hb[:, 2 * KH:]], axis=0)

            def up(w, sm, lo, hi):
                ops = [_upk(sm[j, :, lo]) for j in range(7)]
                rhs = _rhs_ops(ops[:5], ops[5], ops[6])
                rest = [functools.partial(_dot, a, w[2 * KH:D, cols])
                        for a in a5 for cols in (lo, hi)]
                return _strassen(_dot, lhs, rhs, *rest)

            for p in range(npair):
                lo = slice(NW * p, NW * (p + 1))
                hi = slice(FH + NW * p, FH + NW * (p + 1))
                g = up(wg_v, sg, lo, hi)
                u = up(wu_v, su, lo, hi)
                act = [_gelu(g[i]) * u[i] for i in range(4)]
                al = bf16_lhs(*act)
                alo = jnp.concatenate([al[2], act[2].astype(BF16)], axis=0)
                ahi = jnp.concatenate([act[1].astype(BF16), al[3]], axis=0)
                c5 = (c5 + _dot(alo, wd_v[lo, 2 * KH:D])
                      + _dot(ahi, wd_v[hi, 2 * KH:D]))

                def rhs():
                    ops = [_upk(sd[j, _hs(NW * p, NW * (p + 1)), :]) for j in range(7)]
                    return _rhs_ops(ops[:5], ops[5], ops[6])

                if p < npair - 1:
                    cs = _strassen(_dot, al, rhs(), *cs)
                    continue
                for q in range(0, HB, tq):
                    qs = slice(q, q + tq)
                    f11, f12, f21, f22 = _strassen(
                        _dot, [a[qs] for a in al], rhs(), *[c[qs] for c in cs])
                    res = _merge_rows(
                        jnp.concatenate([f11, f12, c5[qs]], axis=1),
                        jnp.concatenate([f21, f22, c5[HB + q:HB + q + tq]], axis=1))
                    r0 = base + 2 * q
                    o_v[pl.ds(pl.multiple_of(r0, 2 * tq), 2 * tq), :] = res.astype(BF16)
                    out_cp(r0, 2 * tq).start()

        def p2_body(t, carry):
            o = jnp.concatenate([att_num(t, b) for b in range(T // 256)], axis=0)
            hs = [att_out(t, r, o[r:r + HB]) for r in range(0, T, HB)]
            for i in range(0, len(hs), 2):
                ffn(t * T + i * HB, hs[i:i + 2], TQ if i + 2 == len(hs) else HB)
            return carry

        lax.fori_loop(0, NT, p2_body, 0)
        pltpu.make_async_copy(o_v, o_hbm, sems.at[0]).wait()

    return kernel, NT


def build(T=512, TQ=64, QF=3, KF=3, NW=256, JC=256,
          PW=(1, 1, 1, 1, 0, 0, 0, 0, 3, 3, 3, 3), PST=32,
          LW=(1, 1, 1, 1), AW=(1, 1), NB=128, VOFF=12,
          MORD=((0, 0), (0, 1), (1, 0), (1, 1))):
    kernel, NT = _make_kernel(T, TQ, QF, KF, NW, JC, PW, PST, LW, AW, NB, VOFF, MORD)

    @jax.jit
    def fn(A_x, A_wqkv, A_w_phi, A_wo, B_x, B_w_gate, B_w_up, B_w_down):
        x = A_x.reshape(S, D)
        wphi = jnp.transpose(A_w_phi, (1, 2, 0))
        any_spec = pl.BlockSpec(memory_space=pl.ANY)
        out = pl.pallas_call(
            kernel,
            in_specs=[any_spec] * 7,
            out_specs=any_spec,
            out_shape=jax.ShapeDtypeStruct((S, D), BF16),
            scratch_shapes=[
                pltpu.VMEM((S, D), BF16),
                pltpu.VMEM((DH, DH, H), BF16),
                pltpu.VMEM((D, D), BF16),
                pltpu.VMEM((D, D), BF16),
                pltpu.VMEM((D, D), BF16),
                pltpu.VMEM((D, D), BF16),
                pltpu.VMEM((D, F), BF16),
                pltpu.VMEM((D, F), BF16),
                pltpu.VMEM((F, D), BF16),
                pltpu.VMEM((3 * D // 2, D), U32),
                pltpu.VMEM((3, 5, DHALF // 2, KH), U32),
                pltpu.VMEM((T // 2, D), U32),
                pltpu.VMEM((7, T // 4, KH), U32),
                pltpu.VMEM((T // 4, 256), U32),
                pltpu.VMEM((NT, D, T), U32),
                pltpu.VMEM((NG, VR, PR), F32),
                pltpu.VMEM((NG, VR // 2, PR), U32),
                pltpu.VMEM((7, KH // 2, FH), U32),
                pltpu.VMEM((7, KH // 2, FH), U32),
                pltpu.VMEM((7, FH // 2, KH), U32),
                pltpu.VMEM((S, D), BF16),
                pltpu.VMEM((2, DHALF, T), U32),
                pltpu.SMEM((1,), U32),
                pltpu.SemaphoreType.DMA((7,)),
            ],
            compiler_params=pltpu.CompilerParams(
                vmem_limit_bytes=100 * 1024 * 1024),
            name="hedgehog_block",
        )(x, A_wqkv, wphi, A_wo, B_w_gate, B_w_up, B_w_down)
        return out.reshape(1, S, D)

    return fn


_impl = build(T=512)


@jax.jit
def pallas_sequential_preLN__linear_kernel_hedgehog__geglu_ffn__prompt_kernel(
    A_x: jax.Array,
    A_wqkv: jax.Array,
    A_w_phi: jax.Array,
    A_wo: jax.Array,
    B_x: jax.Array,
    B_w_gate: jax.Array,
    B_w_up: jax.Array,
    B_w_down: jax.Array,
):
    return _impl(A_x, A_wqkv, A_w_phi, A_wo, B_x, B_w_gate, B_w_up, B_w_down)
```

```python
import functools
import math

import jax
import jax.numpy as jnp
from jax import lax
import jax.experimental.pallas as pl
import jax.experimental.pallas.tpu as pltpu

S, D, H, DH, F = 2048, 640, 32, 20, 1536
NG = 16
GR = 40
PR = 80
VR = 48
DHALF = D // 2
KH = 256
FH = F // 2
HB = 128
PG = 16
T = 512
NT = S // T
TH = T // 2
NW = 256
TQ = 32
KF = 3
PST = 16
GORD = (0, 6, 7, 1, 8, 2, 9, 3, 10, 4, 11, 5, 12, 13, 14, 15)
LN_EPS = 1e-5
DEN_EPS = 1e-6
LOG2E = math.log2(math.e)
F32 = jnp.float32
BF16 = jnp.bfloat16
U32 = jnp.uint32


def _dot(a, b):
    return jnp.dot(a, b, preferred_element_type=F32)


def _dot_nt(a, b):
    return lax.dot_general(a, b, (((1,), (1,)), ((), ())),
                           preferred_element_type=F32)


def _pk(v):
    return pltpu.bitcast(v.astype(BF16), U32)


def _upk(w):
    return pltpu.bitcast(w, BF16)


def _hs(a, b):
    assert a % 16 == 0 and b % 16 == 0
    return slice(a // 2, b // 2)


def _layernorm(x, anchor=None):
    t = x.shape[0]
    s1 = x[:, 0:128]
    for k in range(1, D // 128):
        s1 = s1 + x[:, 128 * k:128 * (k + 1)]
    if anchor is not None:
        s1 = (s1.reshape(t // 8, 8, 128) + anchor[None]).reshape(t, 128)
    mu = jnp.sum(s1, axis=-1, keepdims=True) * (1.0 / D)
    xc = x - mu
    var = jnp.mean(xc * xc, axis=-1, keepdims=True)
    return xc * lax.rsqrt(var + LN_EPS)


def _layernorm_shifted(x):
    c = x[:, 0:1]
    s1 = s2 = None
    for k in range(D // 128):
        d = x[:, 128 * k:128 * (k + 1)] - c
        s1 = d if s1 is None else s1 + d
        s2 = d * d if s2 is None else s2 + d * d
    m1 = jnp.sum(s1, axis=-1, keepdims=True) * (1.0 / D)
    m2 = jnp.sum(s2, axis=-1, keepdims=True) * (1.0 / D)
    var = jnp.maximum(m2 - m1 * m1, 0.0)
    return (x - (c + m1)) * lax.rsqrt(var + LN_EPS)


def _allred(op, t):
    t = op(t, pltpu.roll(t, 2, 1))
    return op(t, pltpu.roll(t, 4, 1))


def _recip(s):
    r = pl.reciprocal(s, approx=True)
    return r * (2.0 - s * r)


def _feature_map(p):
    n, t = p.shape[0] // GR, p.shape[1]
    p4 = p.reshape(n, 5, 8, t)
    mx = _allred(jnp.maximum, jnp.max(p4, axis=1))[:, None]
    mn = _allred(jnp.minimum, jnp.min(p4, axis=1))[:, None]
    ep = jnp.exp2(p4 - mx)
    en = jnp.exp2(mn - p4)
    sp = _allred(jnp.add, jnp.sum(ep, axis=1))[:, None]
    sn = _allred(jnp.add, jnp.sum(en, axis=1))[:, None]
    phi = jnp.concatenate([ep * _recip(sp), en * _recip(sn)], axis=1)
    return phi.reshape(n * PR, t)


def _augment_v(vt):
    n, t = vt.shape[0] // GR, vt.shape[1]
    va = jnp.concatenate([vt.reshape(n, GR, t), jnp.ones((n, 8, t), F32)], axis=1)
    return va.reshape(n * VR, t)


def _gelu(g):
    c = math.sqrt(2.0 / math.pi)
    return 0.5 * g * (1.0 + jnp.tanh(c * (g + 0.044715 * (g * g * g))))


def _lhs_sums(a11, a12, a21, a22):
    return [a11 + a22, a21 + a22, a11 + a12, a21 - a11, a12 - a22]


def _rhs_sums(b11, b12, b21, b22):
    return [b11 + b22, b12 - b22, b21 - b11, b11 + b12, b21 + b22]


def _lhs_ops(s, a11, a22):
    return [s[0], s[1], a11, a22, s[2], s[3], s[4]]


def _rhs_ops(s, b11, b22):
    return [s[0], b11, s[1], s[2], b22, s[3], s[4]]


def _strassen_steps(mm, rest, post, out):
    m2 = mm(2)
    yield
    m4 = mm(4)
    yield
    out[1] = post(1, m2 + m4 + rest[1]())
    yield
    m3 = mm(3)
    yield
    m1 = mm(1)
    yield
    out[2] = post(2, m3 + m1 + rest[2]())
    yield
    m0 = mm(0)
    yield
    c11 = m3 - m4 + m0 + mm(6)
    yield
    out[0] = post(0, c11 + rest[0]())
    yield
    c22 = m2 - m1 + m0 + mm(5)
    yield
    out[3] = post(3, c22 + rest[3]())
    yield


def _strassen(lhs, rhs, rest):
    out = [None] * 4
    for _ in _strassen_steps(lambda i: _dot(lhs[i], rhs[i]), rest,
                             lambda _, c: c, out):
        pass
    return out


def _chain(gens):
    for g in gens:
        yield from g


def _split_rows(a):
    n, c = a.shape
    a4 = a.reshape(n // (2 * PG), 2, PG, c)
    return a4[:, 0].reshape(n // 2, c), a4[:, 1].reshape(n // 2, c)


def _merge_rows(top, bot):
    n, c = top.shape
    both = jnp.stack([top.reshape(n // PG, PG, c), bot.reshape(n // PG, PG, c)],
                     axis=1)
    return both.reshape(2 * n, c)


def _fold_windows():
    wins = []
    for kt in range(5):
        g_lo, g_hi = (128 * kt) // GR, (128 * kt + 127) // GR
        r0 = (g_lo * GR) // 16 * 16
        r1 = -((-(g_hi + 1) * GR) // 16) * 16
        wins.append((r0, r1))
    return wins


def _kernel(x_hbm, wqkv_hbm, wphi_hbm, wo_hbm, wg_hbm, wu_hbm, wd_hbm,
            o_hbm,
            x_v, wphi_v, wk_v, wq_v, wv_v, wo_v, wg_v, wu_v, wd_v,
            wT, wS, xn0, xs, x5, phiq, phik, kvacc, kvb, sg, su, sd, so, o_v,
            zero_s, sems):
    wins = _fold_windows()

    srcs = [
        (wphi_hbm, wphi_v),
        (wqkv_hbm.at[:, D:D + 128 * KF], wk_v.at[:, 0:128 * KF]),
        (x_hbm.at[0:TH], x_v.at[0:TH]),
        (wqkv_hbm.at[:, D + 128 * KF:2 * D], wk_v.at[:, 128 * KF:D]),
        (x_hbm.at[TH:T], x_v.at[TH:T]),
        (wqkv_hbm.at[:, 0:D], wq_v),
        (wqkv_hbm.at[:, 2 * D:3 * D], wv_v),
        (x_hbm.at[T:2 * T], x_v.at[T:2 * T]),
        (x_hbm.at[2 * T:S], x_v.at[2 * T:S]),
        (wo_hbm, wo_v),
        (wg_hbm, wg_v),
        (wu_hbm, wu_v),
        (wd_hbm, wd_v),
    ]
    sem_of = [0, 1, 2, 2, 3, 3, 4, 4, 5, 6, 6, 6, 6]

    def cp(k):
        return pltpu.make_async_copy(srcs[k][0], srcs[k][1], sems.at[sem_of[k]])

    def x_rows(r0, n):
        return x_v[pl.ds(pl.multiple_of(r0, 16), n), :].astype(F32)

    def fold_part(kt, bdts, w_ref):
        return _dot_nt(bdts[kt], w_ref[:, 128 * kt:128 * (kt + 1)])

    def fold_store(base, parts, kts):
        for kt in kts:
            r0, r1 = wins[kt]
            pos = r0
            pieces = []
            if kt > 0:
                p0, p1 = wins[kt - 1]
                pieces.append(parts[kt - 1][r0 - p0:] + parts[kt][:p1 - r0])
                pos = p1
            nxt = wins[kt + 1][0] if kt < 4 else r1
            pieces.append(parts[kt][pos - r0:nxt - r0])
            wT[_hs(base + r0, base + nxt), :] = _pk(
                jnp.concatenate(pieces, axis=0) * LOG2E)

    pace = []

    def note(p):
        pace.append([(p, r, n) for n in range(p.shape[1] // 128)
                     for r in range(0, p.shape[0], PST)])
        return p

    def anchors(npace, count):
        pool = [tl for tiles in pace[-npace:] for tl in tiles]
        zero = zero_s[0]
        cache = {}
        out = []
        for i in range(count):
            k = i * len(pool) // count
            if k not in cache:
                p, r, n = pool[k]
                cache[k] = pltpu.bitcast(
                    p[r:r + 8, 128 * n:128 * (n + 1)], U32) & zero
            out.append(cache[k])
        return out

    def block_sums(specs, sums, npace):
        jobs = [(w, dst, rb, k2, n2, r, c)
                for w, dst, rb, k2, n2 in specs
                for r in range(0, k2, 16) for c in range(0, n2, 128)]
        ans = anchors(npace, len(jobs)) if npace else [None] * len(jobs)
        for an, (w, dst, rb, k2, n2, r, c) in zip(ans, jobs):
            def get(r0, c0, an=None):
                if w.dtype == U32:
                    bits = w[_hs(r0, r0 + 16), c0:c0 + 128]
                    return _upk(bits if an is None else bits | an).astype(F32)
                v = w[r0:r0 + 16, c0:c0 + 128].astype(F32)
                if an is None:
                    return v
                return (v.reshape(2, 8, 128)
                        + pltpu.bitcast(an, F32)[None]).reshape(16, 128)

            top, bot = rb + r, rb + k2 + r
            vals = sums(get(top, c, an), get(top, n2 + c),
                        get(bot, c), get(bot, n2 + c, an))
            for j, v in enumerate(vals):
                dst.at[j][_hs(r, r + 16), c:c + 128] = _pk(v)

    def ln_pair(i, r0, anchor=None):
        xn = _layernorm(x_rows(r0, 2 * PG), anchor)
        lo, hi = xn[:PG], xn[PG:]
        b11, b12 = lo[:, 0:KH], hi[:, 0:KH]
        b21, b22 = lo[:, KH:2 * KH], hi[:, KH:2 * KH]
        rows = _hs(PG * i, PG * (i + 1))
        for j, v in enumerate(_rhs_ops(_rhs_sums(b11, b12, b21, b22), b11, b22)):
            xs.at[j][rows, :] = _pk(v)
        x5[rows, :] = _pk(jnp.concatenate([lo[:, 2 * KH:], hi[:, 2 * KH:]], axis=1))
        return lo, hi

    def ln_next(t, npace):
        for i, an in enumerate(anchors(npace, T // (2 * PG))):
            ln_pair(i, t * T + 2 * PG * i, pltpu.bitcast(an, F32))

    def proj_steps(m, n, post, out):
        top = _hs(m * D, m * D + DHALF)
        bot = _hs(m * D + DHALF, (m + 1) * D)
        tok = _hs(HB * n, HB * (n + 1))
        lhs = _lhs_ops([lambda j=j: wS[m, j] for j in range(5)],
                       lambda: wT[top, 0:KH], lambda: wT[bot, KH:2 * KH])
        rest = [lambda r=r, c=c: _dot_nt(_upk(wT[r, 2 * KH:D]),
                                         _upk(x5[tok, 128 * c:128 * (c + 1)]))
                for r in (top, bot) for c in range(2)]
        return _strassen_steps(
            lambda i: note(_dot_nt(_upk(lhs[i]()), _upk(xs[i, tok, :]))),
            rest, post, out)

    def kv_update(vta, last):
        if last:
            row = lax.broadcasted_iota(jnp.int32, (VR, PR), 0)
            odd = lax.broadcasted_iota(jnp.int32, (VR, PR), 1) & 1
            second = jnp.logical_or(
                jnp.logical_and(row >= DH, row < GR), row >= GR + 4)
            keep = odd == second.astype(jnp.int32)
        for g in range(NG):
            c, gg = divmod(g, 8)
            upd = _dot_nt(vta[c][gg * VR:(gg + 1) * VR, :].astype(BF16),
                          _upk(phik[_hs(g * PR, (g + 1) * PR), :]))
            if last:
                kvb.at[g][...] = _pk(jnp.where(keep, kvacc[g] + upd, 0.0))
            else:
                kvacc[g] += upd

    def w_sums(m, npace):
        block_sums([(wT, wS.at[m], m * D, DHALF, KH)], _lhs_sums, npace)

    pending = []

    def store_phi(dst, n):
        def post(i, c):
            r, hi = divmod(i, 2)
            pending.append((dst, r, TH * hi + HB * n, _feature_map(c)))
        return post

    def flush(which=None):
        keep = []
        for dst, r, l0, phi in pending:
            if which is None or dst is which:
                dst[_hs(D * r, D * (r + 1)), l0:l0 + HB] = _pk(phi)
            else:
                keep.append((dst, r, l0, phi))
        pending[:] = keep

    def p1_run(t, mains, voff, every, skip, extra, last):
        nb = TH // HB
        vout = [[None] * 4 for _ in range(nb)]
        dsts = [phik, phiq.at[t]]
        n0 = len(pace)
        main = _chain([proj_steps(m, n, store_phi(dsts[m], n), [None] * 4)
                       for m, n in mains])
        side = _chain([proj_steps(2, n, lambda i, c: _augment_v(c), vout[n])
                       for n in range(nb)])
        for i, _ in enumerate(main):
            if i + 1 >= voff and i % every == every - 1:
                next(side, None)
        for _ in side:
            pass
        flush(dsts[1])
        extra(len(pace) - n0 - skip)
        flush()
        kv_update([jnp.concatenate([vout[n][2 * r + hi] for hi in range(2)
                                    for n in range(nb)], axis=1)
                   for r in range(2)], last)

    for k in range(len(srcs)):
        cp(k).start()
    zero_s[0] = jnp.uint32(0)
    kvacc[...] = jnp.zeros(kvacc.shape, F32)
    rel = (lax.broadcasted_iota(jnp.int32, (H, D), 1)
           - DH * lax.broadcasted_iota(jnp.int32, (H, D), 0))
    e2 = jnp.where(
        lax.broadcasted_iota(jnp.int32, (VR, DH), 0) >> 1
        == lax.broadcasted_iota(jnp.int32, (VR, DH), 1), 1.0, 0.0).astype(BF16)
    lane8 = lax.broadcasted_iota(jnp.int32, (8, 128), 1)
    sub8 = lax.broadcasted_iota(jnp.int32, (8, 128), 0)
    cp(0).wait()
    m = None
    for d in range(DH):
        sel = jnp.where(rel == d, 1.0, 0.0).astype(BF16)
        t = _dot(wphi_v[d], sel)
        m = t if m is None else m + t
    m2 = _dot(e2, m.astype(BF16))[0:GR]
    relp = lane8 - DH * (sub8 & 1)
    bdts = []
    for kt in range(5):
        r0, r1 = wins[kt]
        pat = m2[:, 128 * kt:128 * (kt + 1)].reshape(5, 8, 128)
        rows = []
        r = r0
        while r < r1:
            g, o = divmod(r, GR)
            n = min(GR - o, r1 - r)
            c0 = GR * g - 128 * kt
            msk = jnp.logical_and(relp >= c0, relp < c0 + DH)
            rows.append(jnp.where(msk[None], pat[o // 8:(o + n) // 8], 0.0))
            r += n
        bdts.append(jnp.concatenate(rows, axis=0)
                    .reshape(r1 - r0, 128).astype(BF16))

    cp(1).wait()
    parts = [fold_part(kt, bdts, wk_v) for kt in range(KF)]
    fold_store(0, parts, range(KF))
    cp(2).wait()
    cp(3).wait()
    for i in range(HB // PG):
        lo, hi = ln_pair(i, 2 * PG * i)
        xn0[_hs(PG * i, PG * (i + 1)), :] = _pk(lo)
        xn0[_hs(HB + PG * i, HB + PG * (i + 1)), :] = _pk(hi)
    parts += [fold_part(kt, bdts, wk_v) for kt in range(KF, 5)]
    fold_store(0, parts, range(KF, 5))
    for r in range(2):
        phi = _feature_map(note(_dot_nt(
            _upk(wT[_hs(DHALF * r, DHALF * (r + 1)), :]), _upk(xn0[...]))))
        for hi in range(2):
            phik[_hs(D * r, D * (r + 1)), TH * hi:TH * hi + HB] = _pk(
                phi[:, HB * hi:HB * (hi + 1)])
    w_sums(0, 2)
    cp(4).wait()
    cp(5).wait()
    for i in range(HB // PG, TH // PG):
        ln_pair(i, 2 * PG * i)
    fold_store(D, [fold_part(kt, bdts, wq_v) for kt in range(5)], range(5))
    for _ in proj_steps(0, 1, store_phi(phik, 1), [None] * 4):
        pass
    flush()
    w_sums(1, 7)
    cp(6).wait()
    cp(7).wait()
    wT[_hs(2 * D, 3 * D), :] = _pk(wv_v[...].T)
    w_sums(2, 0)
    p1_run(0, ((1, 0), (1, 1)), 8, 1, 10, lambda n: ln_next(1, n), False)
    cp(8).wait()

    all_mains = ((0, 0), (0, 1), (1, 0), (1, 1))

    def p1_body(t, carry):
        p1_run(t, all_mains, 12, 2, 0, lambda n: ln_next(t + 1, n), False)
        return carry

    lax.fori_loop(1, NT - 1, p1_body, 0)
    for k in range(9, 13):
        cp(k).wait()
    p1_run(NT - 1, all_mains, 12, 2, 0,
           lambda n: block_sums(
               [(wg_v, sg, 0, KH, FH), (wu_v, su, 0, KH, FH),
                (wd_v, sd, 0, FH, KH), (wo_v, so, 0, KH, KH)], _rhs_sums, n),
           True)

    def att_num(ti, b):
        def phi(g):
            rows = _hs(PR * g, PR * (g + 1))
            return _upk(jnp.concatenate(
                [phiq[ti, rows, c0:c0 + HB] for c0 in (HB * b, TH + HB * b)],
                axis=1))

        gnum = [None] * NG
        for g in GORD:
            gnum[g] = _dot(_upk(kvb[g]), phi(g))
        sub = lax.broadcasted_iota(jnp.int32, (8, 2 * HB), 0) < 4
        pieces = []
        for g in range(NG):
            rec = _recip(gnum[g][GR:VR] + DEN_EPS)
            rot = pltpu.roll(rec, 4, 0)
            ra = jnp.where(sub, rec, rot)
            rb = jnp.where(sub, rot, rec)
            scale = jnp.concatenate([ra, ra, rec, rb, rb], axis=0)
            pieces.append(gnum[g][0:GR] * scale)
        return jnp.concatenate(pieces, axis=0)

    def att_operands(ot):
        o = ot.astype(BF16).T
        sums = _lhs_sums(ot[0:KH, :HB], ot[KH:2 * KH, :HB],
                         ot[0:KH, HB:], ot[KH:2 * KH, HB:])
        st = jnp.concatenate(
            [jnp.concatenate([v[:128], v[128:]], axis=1) for v in sums], axis=0)
        st = st.astype(BF16).T
        return o, [jnp.concatenate([st[:HB, 128 * j:128 * (j + 1)],
                                    st[HB:, 128 * j:128 * (j + 1)]], axis=1)
                   for j in range(5)]

    def att_out(ti, b, o, sums):
        xt, xb = _split_rows(x_rows(ti * T + 2 * HB * b, 2 * HB))
        c5 = _dot(o, wo_v[:, 2 * KH:D])
        r5 = _dot(o[:, 2 * KH:], wo_v[2 * KH:D, 0:2 * KH])
        lhs = _lhs_ops(sums, o[:HB, 0:KH], o[HB:, KH:2 * KH])
        rhs = _rhs_ops([_upk(so[j]) for j in range(5)],
                       wo_v[0:KH, 0:KH], wo_v[KH:2 * KH, KH:2 * KH])
        mm = lambda i: _dot(lhs[i], rhs[i])
        m2, m3, m4, m0 = mm(2), mm(3), mm(4), mm(0)
        c12 = m2 + m4 + r5[:HB, KH:]
        c11 = m3 - m4 + m0 + mm(6) + r5[:HB, :KH]
        ht = xt + jnp.concatenate([c11, c12, c5[:HB]], axis=1)
        m1 = mm(1)
        c21 = m3 + m1 + r5[HB:, :KH]
        c22 = m2 - m1 + m0 + mm(5) + r5[HB:, KH:]
        hb = xb + jnp.concatenate([c21, c22, c5[HB:]], axis=1)
        return (ht, _layernorm_shifted(ht)), (hb, _layernorm_shifted(hb))

    def out_cp(r0, n):
        rows = pl.ds(pl.multiple_of(r0, 16), n)
        return pltpu.make_async_copy(o_v.at[rows], o_hbm.at[rows], sems.at[0])

    def ffn(base, halves, tq):
        (ht, nt_), (hb, nb) = halves
        a11, a22 = nt_[:, 0:KH], nb[:, KH:2 * KH]
        lhs = [v.astype(BF16) for v in _lhs_ops(
            _lhs_sums(a11, nt_[:, KH:2 * KH], nb[:, 0:KH], a22), a11, a22)]
        a5 = [nt_[:, 2 * KH:].astype(BF16), nb[:, 2 * KH:].astype(BF16)]
        cs = [ht[:, 0:KH], ht[:, KH:2 * KH], hb[:, 0:KH], hb[:, KH:2 * KH]]
        c5 = jnp.concatenate([ht[:, 2 * KH:], hb[:, 2 * KH:]], axis=0)

        def up(w, sm, lo, hi):
            rhs = _rhs_ops([_upk(sm[j, :, lo]) for j in range(5)],
                           w[0:KH, lo], w[KH:2 * KH, hi])
            rest = [functools.partial(_dot, a, w[2 * KH:D, cols])
                    for a in a5 for cols in (lo, hi)]
            return _strassen(lhs, rhs, rest)

        for p in range(FH // NW):
            lo = slice(NW * p, NW * (p + 1))
            hi = slice(FH + NW * p, FH + NW * (p + 1))
            g = up(wg_v, sg, lo, hi)
            u = up(wu_v, su, lo, hi)
            act = [_gelu(g[i]) * u[i] for i in range(4)]
            al = _lhs_ops(_lhs_sums(*act), act[0], act[3])
            alo = jnp.concatenate([act[0], act[2]], axis=0).astype(BF16)
            ahi = jnp.concatenate([act[1], act[3]], axis=0).astype(BF16)
            c5 = (c5 + _dot(alo, wd_v[lo, 2 * KH:D])
                  + _dot(ahi, wd_v[hi, 2 * KH:D]))

            def down(rows):
                rhs = _rhs_ops(
                    [_upk(sd[j, _hs(NW * p, NW * (p + 1)), :]) for j in range(5)],
                    wd_v[lo, 0:KH], wd_v[hi, KH:2 * KH])
                return _strassen([a[rows].astype(BF16) for a in al], rhs,
                                 [lambda c=c: c[rows] for c in cs])

            if p < FH // NW - 1:
                cs = down(slice(0, HB))
                continue
            for q in range(0, HB, tq):
                f11, f12, f21, f22 = down(slice(q, q + tq))
                res = _merge_rows(
                    jnp.concatenate([f11, f12, c5[q:q + tq]], axis=1),
                    jnp.concatenate([f21, f22, c5[HB + q:HB + q + tq]], axis=1))
                r0 = base + 2 * q
                o_v[pl.ds(pl.multiple_of(r0, 2 * tq), 2 * tq), :] = res.astype(BF16)
                out_cp(r0, 2 * tq).start()

    def p2_body(t, carry):
        nb = TH // HB
        ops = [att_operands(att_num(t, b)) for b in range(nb)]
        hs = [att_out(t, b, *ops[b]) for b in range(nb)]
        for b in range(nb):
            ffn(t * T + 2 * HB * b, hs[b], TQ if b + 1 == nb else HB)
        return carry

    lax.fori_loop(0, NT, p2_body, 0)
    pltpu.make_async_copy(o_v, o_hbm, sems.at[0]).wait()


@jax.jit
def pallas_sequential_preLN__linear_kernel_hedgehog__geglu_ffn__prompt_kernel(
    A_x: jax.Array,
    A_wqkv: jax.Array,
    A_w_phi: jax.Array,
    A_wo: jax.Array,
    B_x: jax.Array,
    B_w_gate: jax.Array,
    B_w_up: jax.Array,
    B_w_down: jax.Array,
):
    del B_x
    x = A_x.reshape(S, D)
    wphi = jnp.transpose(A_w_phi, (1, 2, 0))
    any_spec = pl.BlockSpec(memory_space=pl.ANY)
    out = pl.pallas_call(
        _kernel,
        in_specs=[any_spec] * 7,
        out_specs=any_spec,
        out_shape=jax.ShapeDtypeStruct((S, D), BF16),
        scratch_shapes=[
            pltpu.VMEM((S, D), BF16),
            pltpu.VMEM((DH, DH, H), BF16),
            pltpu.VMEM((D, D), BF16),
            pltpu.VMEM((D, D), BF16),
            pltpu.VMEM((D, D), BF16),
            pltpu.VMEM((D, D), BF16),
            pltpu.VMEM((D, F), BF16),
            pltpu.VMEM((D, F), BF16),
            pltpu.VMEM((F, D), BF16),
            pltpu.VMEM((3 * D // 2, D), U32),
            pltpu.VMEM((3, 5, DHALF // 2, KH), U32),
            pltpu.VMEM((HB, D), U32),
            pltpu.VMEM((7, TH // 2, KH), U32),
            pltpu.VMEM((TH // 2, 256), U32),
            pltpu.VMEM((NT, D, T), U32),
            pltpu.VMEM((D, T), U32),
            pltpu.VMEM((NG, VR, PR), F32),
            pltpu.VMEM((NG, VR // 2, PR), U32),
            pltpu.VMEM((5, KH // 2, FH), U32),
            pltpu.VMEM((5, KH // 2, FH), U32),
            pltpu.VMEM((5, FH // 2, KH), U32),
            pltpu.VMEM((5, KH // 2, KH), U32),
            pltpu.VMEM((S, D), BF16),
            pltpu.SMEM((1,), U32),
            pltpu.SemaphoreType.DMA((7,)),
        ],
        compiler_params=pltpu.CompilerParams(
            vmem_limit_bytes=100 * 1024 * 1024),
        name="hedgehog_block",
    )(x, A_wqkv, wphi, A_wo, B_w_gate, B_w_up, B_w_down)
    return out.reshape(1, S, D)
```

```python
import functools
import math

import jax
import jax.numpy as jnp
from jax import lax
import jax.experimental.pallas as pl
import jax.experimental.pallas.tpu as pltpu

S, D, H, DH, F = 2048, 640, 32, 20, 1536
NG = 16
GR = 40
PR = 80
VR = 48
DHALF = D // 2
KH = 256
FH = F // 2
HB = 128
PG = 16
T = 512
NT = S // T
TH = T // 2
NW = 256
TQ = 32
KF = 3
LAG = 0
LNR = 32
KVG = 14
KVW = 2
NSH = 42
LN0 = 98
LN1 = 147
PST = 16
GORD = (0, 6, 7, 1, 8, 2, 9, 3, 10, 4, 11, 5, 12, 13, 14, 15)
LN_EPS = 1e-5
DEN_EPS = 1e-6
LOG2E = math.log2(math.e)
F32 = jnp.float32
BF16 = jnp.bfloat16
U32 = jnp.uint32


def _dot(a, b):
    return jnp.dot(a, b, preferred_element_type=F32)


def _dot_nt(a, b):
    return lax.dot_general(a, b, (((1,), (1,)), ((), ())),
                           preferred_element_type=F32)


def _pk(v):
    return pltpu.bitcast(v.astype(BF16), U32)


def _upk(w):
    return pltpu.bitcast(w, BF16)


def _hs(a, b):
    assert a % 16 == 0 and b % 16 == 0
    return slice(a // 2, b // 2)


def _layernorm(x, anchor=None):
    t = x.shape[0]
    s1 = x[:, 0:128]
    for k in range(1, D // 128):
        s1 = s1 + x[:, 128 * k:128 * (k + 1)]
    if anchor is not None:
        s1 = (s1.reshape(t // 8, 8, 128) + anchor[None]).reshape(t, 128)
    mu = jnp.sum(s1, axis=-1, keepdims=True) * (1.0 / D)
    xc = x - mu
    var = jnp.mean(xc * xc, axis=-1, keepdims=True)
    return xc * lax.rsqrt(var + LN_EPS)


def _layernorm_shifted(x, zeros=None):
    c = x[:, 0:128] if zeros is None else x[:, 0:128] + zeros
    c = c[:, 0:1]
    s1 = s2 = None
    for k in range(D // 128):
        d = x[:, 128 * k:128 * (k + 1)] - c
        s1 = d if s1 is None else s1 + d
        s2 = d * d if s2 is None else s2 + d * d
    m1 = jnp.sum(s1, axis=-1, keepdims=True) * (1.0 / D)
    m2 = jnp.sum(s2, axis=-1, keepdims=True) * (1.0 / D)
    var = jnp.maximum(m2 - m1 * m1, 0.0)
    return (x - (c + m1)) * lax.rsqrt(var + LN_EPS)


def _allred(op, t):
    t = op(t, pltpu.roll(t, 2, 1))
    return op(t, pltpu.roll(t, 4, 1))


def _recip(s):
    r = pl.reciprocal(s, approx=True)
    return r * (2.0 - s * r)


def _feature_map(p):
    n, t = p.shape[0] // GR, p.shape[1]
    p4 = p.reshape(n, 5, 8, t)
    mx = _allred(jnp.maximum, jnp.max(p4, axis=1))[:, None]
    mn = _allred(jnp.minimum, jnp.min(p4, axis=1))[:, None]
    ep = jnp.exp2(p4 - mx)
    en = jnp.exp2(mn - p4)
    sp = _allred(jnp.add, jnp.sum(ep, axis=1))[:, None]
    sn = _allred(jnp.add, jnp.sum(en, axis=1))[:, None]
    phi = jnp.concatenate([ep * _recip(sp), en * _recip(sn)], axis=1)
    return phi.reshape(n * PR, t)


def _augment_v(vt):
    n, t = vt.shape[0] // GR, vt.shape[1]
    va = jnp.concatenate([vt.reshape(n, GR, t), jnp.ones((n, 8, t), F32)], axis=1)
    return va.reshape(n * VR, t)


def _gelu(g):
    c = math.sqrt(2.0 / math.pi)
    return 0.5 * g * (1.0 + jnp.tanh(c * (g + 0.044715 * (g * g * g))))


def _lhs_sums(a11, a12, a21, a22):
    return [a11 + a22, a21 + a22, a11 + a12, a21 - a11, a12 - a22]


def _rhs_sums(b11, b12, b21, b22):
    return [b11 + b22, b12 - b22, b21 - b11, b11 + b12, b21 + b22]


def _lhs_ops(s, a11, a22):
    return [s[0], s[1], a11, a22, s[2], s[3], s[4]]


def _rhs_ops(s, b11, b22):
    return [s[0], b11, s[1], s[2], b22, s[3], s[4]]


def _strassen_steps(mm, rest, post, out):
    m2 = mm(2)
    yield
    m4 = mm(4)
    yield
    out[1] = post(1, m2 + m4 + rest[1]())
    yield
    m3 = mm(3)
    yield
    m1 = mm(1)
    yield
    out[2] = post(2, m3 + m1 + rest[2]())
    yield
    m0 = mm(0)
    yield
    c11 = m3 - m4 + m0 + mm(6)
    yield
    out[0] = post(0, c11 + rest[0]())
    yield
    c22 = m2 - m1 + m0 + mm(5)
    yield
    out[3] = post(3, c22 + rest[3]())
    yield


def _run(mm, rest):
    out = [None] * 4
    for _ in _strassen_steps(mm, rest, lambda _, c: c, out):
        pass
    return out


def _quad(a):
    h, k = a.shape[0] // 2, a.shape[1] // 2
    return a[:h, :k], a[:h, k:], a[h:, :k], a[h:, k:]


def _join(c):
    return jnp.concatenate([jnp.concatenate(c[0:2], axis=1),
                            jnp.concatenate(c[2:4], axis=1)], axis=0)


def _lhs7(b):
    return _lhs_ops(_lhs_sums(*b), b[0], b[3])


def _rhs7(b):
    return _rhs_ops(_rhs_sums(*b), b[0], b[3])


def _add_tile(a, z):
    if z is None:
        return a
    r, c = a.shape
    z = jnp.concatenate([z] * (c // 128), axis=1)
    return (a.reshape(r // 8, 8, c) + z[None]).reshape(r, c)


def _lhs_row(b, i, z=None):
    a11, a12, a21, a22 = b
    if i in (2, 3):
        q = list(_quad(a11 if i == 2 else a22))
        q[0], q[3] = _add_tile(q[0], z), _add_tile(q[3], z)
        return _lhs7(q)
    x, y, sign = {0: (a11, a22, 1), 1: (a21, a22, 1), 4: (a11, a12, 1),
                  5: (a21, a11, -1), 6: (a12, a22, -1)}[i]
    x = _add_tile(x, z)
    return _lhs7(_quad(x + y if sign > 0 else x - y))


def _run_late22(mm, rest, mid):
    m2, m4 = mm(2), mm(4)
    c12 = m2 + m4 + rest[1]()
    c22 = m2 + mm(5) + rest[3]()
    mid()
    m3, m1 = mm(3), mm(1)
    c21 = m3 + m1 + rest[2]()
    m0 = mm(0)
    c22 = c22 - m1 + m0
    c11 = m3 - m4 + m0 + mm(6) + rest[0]()
    return [c11, c12, c21, c22]


def _strassen2(lhs_row, rhs, rest, mid=None, plag=3, log=None):
    none = [lambda: 0.0] * 4
    seen = []

    def mm(i):
        ops = lhs_row(i, seen[-plag] if len(seen) >= plag else None)
        first = []

        def inner(j):
            m = _dot(ops[j], rhs(i, j))
            first.append(m)
            return m

        out = _join(_run(inner, none))
        seen.append(first[0][0:8, :])
        if log is not None:
            log.extend(first)
        return out

    return _run(mm, rest) if mid is None else _run_late22(mm, rest, mid)


def _chain(gens):
    for g in gens:
        yield from g


def _split_rows(a):
    n, c = a.shape
    a4 = a.reshape(n // (2 * PG), 2, PG, c)
    return a4[:, 0].reshape(n // 2, c), a4[:, 1].reshape(n // 2, c)


def _merge_rows(top, bot):
    n, c = top.shape
    both = jnp.stack([top.reshape(n // PG, PG, c), bot.reshape(n // PG, PG, c)],
                     axis=1)
    return both.reshape(2 * n, c)


def _fold_windows():
    wins = []
    for kt in range(5):
        g_lo, g_hi = (128 * kt) // GR, (128 * kt + 127) // GR
        r0 = (g_lo * GR) // 16 * 16
        r1 = -((-(g_hi + 1) * GR) // 16) * 16
        wins.append((r0, r1))
    return wins


def _kernel(x_hbm, wqkv_hbm, wphi_hbm, wo_hbm, wg_hbm, wu_hbm, wd_hbm,
            o_hbm,
            x_v, wphi_v, wk_v, wq_v, wv_v, wo_v, wgu_v, wd_v,
            wT, wS, xn0, xs, x5, phiq, phik, kvacc, kvb, sgu, sd, so, o_v,
            zero_s, sems):
    wins = _fold_windows()

    srcs = [
        (wphi_hbm, wphi_v),
        (wqkv_hbm.at[:, D:D + 128 * KF], wk_v.at[:, 0:128 * KF]),
        (x_hbm.at[0:TH], x_v.at[0:TH]),
        (wqkv_hbm.at[:, D + 128 * KF:2 * D], wk_v.at[:, 128 * KF:D]),
        (x_hbm.at[TH:T], x_v.at[TH:T]),
        (wqkv_hbm.at[:, 0:D], wq_v),
        (wqkv_hbm.at[:, 2 * D:3 * D], wv_v),
        (x_hbm.at[T:2 * T], x_v.at[T:2 * T]),
        (x_hbm.at[2 * T:S], x_v.at[2 * T:S]),
        (wg_hbm, wgu_v.at[0]),
        (wu_hbm, wgu_v.at[1]),
        (wo_hbm, wo_v),
        (wd_hbm, wd_v),
    ]
    sem_of = [0, 1, 2, 2, 3, 3, 4, 4, 5, 5, 6, 7, 7]

    def cp(k):
        return pltpu.make_async_copy(srcs[k][0], srcs[k][1], sems.at[sem_of[k]])

    def x_rows(r0, n):
        return x_v[pl.ds(pl.multiple_of(r0, 16), n), :].astype(F32)

    def fold_part(kt, bdts, w_ref):
        return _dot_nt(bdts[kt], w_ref[:, 128 * kt:128 * (kt + 1)])

    def fold_store(base, parts, kts):
        for kt in kts:
            r0, r1 = wins[kt]
            pos = r0
            pieces = []
            if kt > 0:
                p0, p1 = wins[kt - 1]
                pieces.append(parts[kt - 1][r0 - p0:] + parts[kt][:p1 - r0])
                pos = p1
            nxt = wins[kt + 1][0] if kt < 4 else r1
            pieces.append(parts[kt][pos - r0:nxt - r0])
            wT[_hs(base + r0, base + nxt), :] = _pk(
                jnp.concatenate(pieces, axis=0) * LOG2E)

    pace = []

    def note(p):
        pace.append([(p, r, n) for n in range(p.shape[1] // 128)
                     for r in range(0, p.shape[0], PST)])
        return p

    def anchors(npace, count, phase=0.0):
        pool = [tl for tiles in pace[-npace:] for tl in tiles]
        zero = zero_s[0]
        cache = {}
        out = []
        for i in range(count):
            k = int((i + phase) * len(pool) / count)
            if k not in cache:
                p, r, n = pool[k]
                tile = (p[r:r + 8, 128 * n:128 * (n + 1)] if n >= 0 else
                        jnp.broadcast_to(p[r:r + 8, 0:1], (8, 128)))
                cache[k] = pltpu.bitcast(tile, U32) & zero
            out.append(cache[k])
        return out

    def block_sums(specs, sums, npace):
        jobs = [(w, dst, rb, k2, n2, r, c)
                for w, dst, rb, k2, n2 in specs
                for r in range(0, k2, 16) for c in range(0, n2, 128)]
        ans = anchors(npace, len(jobs)) if npace else [None] * len(jobs)
        for an, (w, dst, rb, k2, n2, r, c) in zip(ans, jobs):
            def get(r0, c0, an=None):
                if w.dtype == U32:
                    bits = w[_hs(r0, r0 + 16), c0:c0 + 128]
                    return _upk(bits if an is None else bits | an).astype(F32)
                v = w[r0:r0 + 16, c0:c0 + 128].astype(F32)
                if an is None:
                    return v
                return (v.reshape(2, 8, 128)
                        + pltpu.bitcast(an, F32)[None]).reshape(16, 128)

            top, bot = rb + r, rb + k2 + r
            vals = sums(get(top, c, an), get(top, n2 + c),
                        get(bot, c), get(bot, n2 + c, an))
            for j, v in enumerate(vals):
                dst.at[j][_hs(r, r + 16), c:c + 128] = _pk(v)

    def ffn_sums_jobs(w, dst, up):
        def job(p, r, i, an):
            model = [128 * k for k in range(4)]
            ffn = [NW * p, NW * p + 128, FH + NW * p, FH + NW * p + 128]
            rws, cls = (model, ffn) if up else (ffn, model)
            z = pltpu.bitcast(an, F32)[None]

            def blk(bi, bj):
                return lambda: jnp.concatenate(
                    [w[rws[2 * bi + k] + r:rws[2 * bi + k] + r + 16,
                       cls[2 * bj]:cls[2 * bj] + 256].astype(F32)
                     for k in range(2)], axis=0)

            b11, b12, b21, b22 = blk(0, 0), blk(0, 1), blk(1, 0), blk(1, 1)
            op = [lambda: b11() + b22(), b11, lambda: b12() - b22(),
                  lambda: b21() - b11(), b22, lambda: b11() + b12(),
                  lambda: b21() + b22()][i]()
            q = list(_quad(op))
            for k in (0, 3):
                q[k] = (q[k].reshape(2, 8, 128) + z).reshape(16, 128)
            r0, c0 = (r, 128 * p) if up else (128 * p + r, 0)
            for j, v in enumerate(_rhs7(q)):
                dst.at[7 * i + j][_hs(r0, r0 + 16), c0:c0 + 128] = _pk(v)

        return [functools.partial(job, p, r, i) for p in range(FH // NW)
                for r in range(0, 128, 16) for i in range(7)]

    def run_jobs(jobs, npace):
        for an, job in zip(anchors(npace, len(jobs), 0.5), jobs):
            job(an)

    def ln_pair(i, r0, anchor=None):
        xn = _layernorm(x_rows(r0, 2 * PG), anchor)
        lo, hi = xn[:PG], xn[PG:]
        b11, b12 = lo[:, 0:KH], hi[:, 0:KH]
        b21, b22 = lo[:, KH:2 * KH], hi[:, KH:2 * KH]
        rows = _hs(PG * i, PG * (i + 1))
        for j, v in enumerate(_rhs_ops(_rhs_sums(b11, b12, b21, b22), b11, b22)):
            xs.at[j][rows, :] = _pk(v)
        x5[rows, :] = _pk(jnp.concatenate([lo[:, 2 * KH:], hi[:, 2 * KH:]], axis=1))
        return lo, hi

    def ln_next(t, npace):
        for i, an in enumerate(anchors(npace, T // (2 * PG))):
            ln_pair(i, t * T + 2 * PG * i, pltpu.bitcast(an, F32))

    def proj_steps(m, n, post, out):
        top = _hs(m * D, m * D + DHALF)
        bot = _hs(m * D + DHALF, (m + 1) * D)
        tok = _hs(HB * n, HB * (n + 1))
        lhs = _lhs_ops([lambda j=j: wS[m, j] for j in range(5)],
                       lambda: wT[top, 0:KH], lambda: wT[bot, KH:2 * KH])
        rest = [lambda r=r, c=c: _dot_nt(_upk(wT[r, 2 * KH:D]),
                                         _upk(x5[tok, 128 * c:128 * (c + 1)]))
                for r in (top, bot) for c in range(2)]
        return _strassen_steps(
            lambda i: note(_dot_nt(_upk(lhs[i]()), _upk(xs[i, tok, :]))),
            rest, post, out)

    def kv_update(vta, last):
        if last:
            row = lax.broadcasted_iota(jnp.int32, (VR, PR), 0)
            odd = lax.broadcasted_iota(jnp.int32, (VR, PR), 1) & 1
            second = jnp.logical_or(
                jnp.logical_and(row >= DH, row < GR), row >= GR + 4)
            keep = odd == second.astype(jnp.int32)
        for g in range(NG):
            c, gg = divmod(g, 8)
            upd = _dot_nt(vta[c][gg * VR:(gg + 1) * VR, :].astype(BF16),
                          _upk(phik[_hs(g * PR, (g + 1) * PR), :]))
            if g < KVG:
                pace.append([(upd, r, -1) for r in range(0, VR, 8)
                             for _ in range(KVW)])
            if last:
                kvb.at[g][...] = _pk(jnp.where(keep, kvacc[g] + upd, 0.0))
            else:
                kvacc[g] += upd

    def w_sums(m, npace):
        block_sums([(wT, wS.at[m], m * D, DHALF, KH)], _lhs_sums, npace)

    pending = []

    def store_phi(dst, n):
        def post(i, c):
            r, hi = divmod(i, 2)
            pending.append((dst, r, TH * hi + HB * n, _feature_map(c)))
        return post

    def flush(which=None):
        keep = []
        for dst, r, l0, phi in pending:
            if which is None or dst is which:
                dst[_hs(D * r, D * (r + 1)), l0:l0 + HB] = _pk(phi)
            else:
                keep.append((dst, r, l0, phi))
        pending[:] = keep

    def p1_run(t, mains, voff, every, skip, extra, last, late=None):
        nb = TH // HB
        vout = [[None] * 4 for _ in range(nb)]
        dsts = [phik, phiq.at[t]]
        n0 = len(pace)
        main = _chain([proj_steps(m, n, store_phi(dsts[m], n), [None] * 4)
                       for m, n in mains])
        side = _chain([proj_steps(2, n, lambda i, c: _augment_v(c), vout[n])
                       for n in range(nb)])
        for i, _ in enumerate(main):
            if i + 1 >= voff and i % every == every - 1:
                next(side, None)
        for _ in side:
            pass
        flush(dsts[1])
        extra(len(pace) - n0 - skip)
        flush()
        kv_update([jnp.concatenate([vout[n][2 * r + hi] for hi in range(2)
                                    for n in range(nb)], axis=1)
                   for r in range(2)], last)
        if late is not None:
            late(len(pace) - n0)

    for k in range(len(srcs)):
        cp(k).start()
    zero_s[0] = jnp.uint32(0)
    kvacc[...] = jnp.zeros(kvacc.shape, F32)
    rel = (lax.broadcasted_iota(jnp.int32, (H, D), 1)
           - DH * lax.broadcasted_iota(jnp.int32, (H, D), 0))
    e2 = jnp.where(
        lax.broadcasted_iota(jnp.int32, (VR, DH), 0) >> 1
        == lax.broadcasted_iota(jnp.int32, (VR, DH), 1), 1.0, 0.0).astype(BF16)
    lane8 = lax.broadcasted_iota(jnp.int32, (8, 128), 1)
    sub8 = lax.broadcasted_iota(jnp.int32, (8, 128), 0)
    cp(0).wait()
    m = None
    for d in range(DH):
        sel = jnp.where(rel == d, 1.0, 0.0).astype(BF16)
        t = _dot(wphi_v[d], sel)
        m = t if m is None else m + t
    m2 = _dot(e2, m.astype(BF16))[0:GR]
    relp = lane8 - DH * (sub8 & 1)
    bdts = []
    for kt in range(5):
        r0, r1 = wins[kt]
        pat = m2[:, 128 * kt:128 * (kt + 1)].reshape(5, 8, 128)
        rows = []
        r = r0
        while r < r1:
            g, o = divmod(r, GR)
            n = min(GR - o, r1 - r)
            c0 = GR * g - 128 * kt
            msk = jnp.logical_and(relp >= c0, relp < c0 + DH)
            rows.append(jnp.where(msk[None], pat[o // 8:(o + n) // 8], 0.0))
            r += n
        bdts.append(jnp.concatenate(rows, axis=0)
                    .reshape(r1 - r0, 128).astype(BF16))

    cp(1).wait()
    parts = [fold_part(kt, bdts, wk_v) for kt in range(KF)]
    fold_store(0, parts, range(KF))
    cp(2).wait()
    cp(3).wait()
    for i in range(HB // PG):
        lo, hi = ln_pair(i, 2 * PG * i)
        xn0[_hs(PG * i, PG * (i + 1)), :] = _pk(lo)
        xn0[_hs(HB + PG * i, HB + PG * (i + 1)), :] = _pk(hi)
    parts += [fold_part(kt, bdts, wk_v) for kt in range(KF, 5)]
    fold_store(0, parts, range(KF, 5))
    for r in range(2):
        phi = _feature_map(note(_dot_nt(
            _upk(wT[_hs(DHALF * r, DHALF * (r + 1)), :]), _upk(xn0[...]))))
        for hi in range(2):
            phik[_hs(D * r, D * (r + 1)), TH * hi:TH * hi + HB] = _pk(
                phi[:, HB * hi:HB * (hi + 1)])
    w_sums(0, 2)
    cp(4).wait()
    cp(5).wait()
    for i in range(HB // PG, TH // PG):
        ln_pair(i, 2 * PG * i)
    fold_store(D, [fold_part(kt, bdts, wq_v) for kt in range(5)], range(5))
    for _ in proj_steps(0, 1, store_phi(phik, 1), [None] * 4):
        pass
    flush()
    w_sums(1, 7)
    cp(6).wait()
    cp(7).wait()
    wT[_hs(2 * D, 3 * D), :] = _pk(wv_v[...].T)
    w_sums(2, 0)
    p1_run(0, ((1, 0), (1, 1)), 8, 1, 10, lambda n: ln_next(1, n), False)
    cp(8).wait()
    cp(9).wait()

    all_mains = ((0, 0), (0, 1), (1, 0), (1, 1))

    def p1_body(t, carry):
        @pl.when(t == 2)
        def _():
            cp(10).wait()

        p1_run(t, all_mains, 12, 2, 0, lambda n: ln_next(t + 1, n), False,
               lambda n: run_jobs(
                   ffn_sums_jobs(wgu_v.at[t - 1], sgu.at[t - 1], True)[NSH:], n))
        return carry

    lax.fori_loop(1, NT - 1, p1_body, 0)
    cp(11).wait()
    cp(12).wait()

    p1_run(NT - 1, all_mains, 12, 2, 0,
           lambda n: block_sums([(wo_v, so, 0, KH, KH)], _rhs_sums, n), True,
           lambda n: run_jobs(
               ffn_sums_jobs(wgu_v.at[0], sgu.at[0], True)[:NSH]
               + ffn_sums_jobs(wgu_v.at[1], sgu.at[1], True)[:NSH]
               + ffn_sums_jobs(wd_v, sd, False), n))

    def att_num(ti, b):
        def phi(g):
            rows = _hs(PR * g, PR * (g + 1))
            return _upk(jnp.concatenate(
                [phiq[ti, rows, c0:c0 + HB] for c0 in (HB * b, TH + HB * b)],
                axis=1))

        gnum = [None] * NG
        for g in GORD:
            gnum[g] = _dot(_upk(kvb[g]), phi(g))
        sub = lax.broadcasted_iota(jnp.int32, (8, 2 * HB), 0) < 4
        pieces = []
        for g in range(NG):
            rec = _recip(gnum[g][GR:VR] + DEN_EPS)
            rot = pltpu.roll(rec, 4, 0)
            ra = jnp.where(sub, rec, rot)
            rb = jnp.where(sub, rot, rec)
            scale = jnp.concatenate([ra, ra, rec, rb, rb], axis=0)
            pieces.append(gnum[g][0:GR] * scale)
        return jnp.concatenate(pieces, axis=0)

    def att_operands(ot):
        o = ot.astype(BF16).T
        sums = _lhs_sums(ot[0:KH, :HB], ot[KH:2 * KH, :HB],
                         ot[0:KH, HB:], ot[KH:2 * KH, HB:])
        st = jnp.concatenate(
            [jnp.concatenate([v[:128], v[128:]], axis=1) for v in sums], axis=0)
        st = st.astype(BF16).T
        return o, [jnp.concatenate([st[:HB, 128 * j:128 * (j + 1)],
                                    st[HB:, 128 * j:128 * (j + 1)]], axis=1)
                   for j in range(5)]

    def att_out(ti, b, o, sums):
        xt, xb = _split_rows(x_rows(ti * T + 2 * HB * b, 2 * HB))
        c5 = _dot(o, wo_v[:, 2 * KH:D])
        r5 = _dot(o[:, 2 * KH:], wo_v[2 * KH:D, 0:2 * KH])
        lhs = _lhs_ops(sums, o[:HB, 0:KH], o[HB:, KH:2 * KH])
        rhs = _rhs_ops([_upk(so[j]) for j in range(5)],
                       wo_v[0:KH, 0:KH], wo_v[KH:2 * KH, KH:2 * KH])
        mm = lambda i: _dot(lhs[i], rhs[i])
        m2, m3, m4, m0 = mm(2), mm(3), mm(4), mm(0)
        c12 = m2 + m4 + r5[:HB, KH:]
        c11 = m3 - m4 + m0 + mm(6) + r5[:HB, :KH]
        ht = xt + jnp.concatenate([c11, c12, c5[:HB]], axis=1)
        m1 = mm(1)
        c21 = m3 + m1 + r5[HB:, :KH]
        c22 = m2 - m1 + m0 + mm(5) + r5[HB:, KH:]
        hb = xb + jnp.concatenate([c21, c22, c5[HB:]], axis=1)
        return ht, hb

    def out_cp(r0, n):
        rows = pl.ds(pl.multiple_of(r0, 16), n)
        return pltpu.make_async_copy(o_v.at[rows], o_hbm.at[rows], sems.at[0])

    def zero_of(tile):
        if tile is None:
            return None
        return pltpu.bitcast(pltpu.bitcast(tile, U32) & zero_s[0], F32)

    class Ffn:
        def __init__(self, base, halves, tq, tiles=None):
            ht, hb = halves
            zs = [None, None]
            if tiles is not None:
                n = HB // LNR
                pick = [zero_of(tiles[k * len(tiles) // n][0:8, :]) for k in range(n)]
                zs = [jnp.concatenate([z for z in pick for _ in range(LNR // 8)],
                                      axis=0)] * 2
            nt_, nb = _layernorm_shifted(ht, zs[0]), _layernorm_shifted(hb, zs[1])
            self.log = []
            self.base, self.tq = base, tq
            self.hn = (nt_[:, 0:KH], nt_[:, KH:2 * KH], nb[:, 0:KH], nb[:, KH:2 * KH])
            self.lhs = {}
            self.a5 = [nt_[:, 2 * KH:].astype(BF16), nb[:, 2 * KH:].astype(BF16)]
            self.cs = [ht[:, 0:KH], ht[:, KH:2 * KH], hb[:, 0:KH], hb[:, KH:2 * KH]]
            self.c5 = jnp.concatenate([ht[:, 2 * KH:], hb[:, 2 * KH:]], axis=0)
            self.act = {}

        def up(self, p):
            cols = (slice(NW * p, NW * (p + 1)), slice(FH + NW * p, FH + NW * (p + 1)))

            def proj(m):
                rest = [functools.partial(_dot, a, wgu_v[m, 2 * KH:D, c])
                        for a in self.a5 for c in cols]
                def lhs_row(i, tile):
                    if i not in self.lhs:
                        self.lhs[i] = [v.astype(BF16) for v in
                                       _lhs_row(self.hn, i, zero_of(tile))]
                    return self.lhs[i]

                return _strassen2(
                    lhs_row,
                    lambda i, j: _upk(sgu[m, 7 * i + j, :, 128 * p:128 * (p + 1)]),
                    rest, log=self.log)

            g, u = proj(0), proj(1)
            self.act[p] = [_gelu(g[i]) * u[i] for i in range(4)]

        def down(self, p):
            act = self.act.pop(p)

            def last_tile(k):
                a = jnp.concatenate([act[k], act[2 + k]], axis=0).astype(BF16)
                r0 = FH * k + NW * p
                self.c5 = self.c5 + _dot(a, wd_v[r0:r0 + NW, 2 * KH:D])

            last_tile(0)
            rhs = lambda i, j: _upk(sd[7 * i + j, _hs(128 * p, 128 * (p + 1)), 0:128])
            if p < FH // NW - 1:
                self.cs = _strassen2(
                    lambda i, tile: [v.astype(BF16) for v in
                                     _lhs_row(act, i, zero_of(tile))],
                    rhs, [lambda c=c: c for c in self.cs], lambda: last_tile(1))
                return
            tq, hq = self.tq, HB // 2
            for q in range(0, hq, tq):
                pick = lambda c: jnp.concatenate(
                    [c[q:q + tq], c[hq + q:hq + q + tq]], axis=0)
                sub = [pick(a) for a in act]
                f = _strassen2(lambda i, tile: [v.astype(BF16) for v in
                                                _lhs_row(sub, i, zero_of(tile))],
                               rhs,
                               [lambda c=c: pick(c) for c in self.cs],
                               lambda: last_tile(1) if q == 0 else None,
                               plag=3 * hq // tq)
                top = jnp.concatenate([f[0], f[1], pick(self.c5[:HB])], axis=1)
                bot = jnp.concatenate([f[2], f[3], pick(self.c5[HB:])], axis=1)
                for k in range(2):
                    res = _merge_rows(top[tq * k:tq * (k + 1)], bot[tq * k:tq * (k + 1)])
                    r0 = self.base + 2 * (hq * k + q)
                    o_v[pl.ds(pl.multiple_of(r0, 2 * tq), 2 * tq), :] = res.astype(BF16)
                    out_cp(r0, 2 * tq).start()

    def p2_body(t, carry):
        nb = TH // HB
        ops = [att_operands(att_num(t, b)) for b in range(nb)]
        hs = [att_out(t, b, *ops[b]) for b in range(nb)]
        tiles = None
        for b in range(nb):
            f = Ffn(t * T + 2 * HB * b, hs[b], TQ if b + 1 == nb else HB // 2, tiles)
            for p in range(FH // NW):
                f.up(p)
                f.down(p)
            tiles = f.log[LN0:LN1]
        return carry

    lax.fori_loop(0, NT, p2_body, 0)
    pltpu.make_async_copy(o_v, o_hbm, sems.at[0]).wait()


@jax.jit
def pallas_sequential_preLN__linear_kernel_hedgehog__geglu_ffn__prompt_kernel(
    A_x: jax.Array,
    A_wqkv: jax.Array,
    A_w_phi: jax.Array,
    A_wo: jax.Array,
    B_x: jax.Array,
    B_w_gate: jax.Array,
    B_w_up: jax.Array,
    B_w_down: jax.Array,
):
    del B_x
    x = A_x.reshape(S, D)
    wphi = jnp.transpose(A_w_phi, (1, 2, 0))
    any_spec = pl.BlockSpec(memory_space=pl.ANY)
    out = pl.pallas_call(
        _kernel,
        in_specs=[any_spec] * 7,
        out_specs=any_spec,
        out_shape=jax.ShapeDtypeStruct((S, D), BF16),
        scratch_shapes=[
            pltpu.VMEM((S, D), BF16),
            pltpu.VMEM((DH, DH, H), BF16),
            pltpu.VMEM((D, D), BF16),
            pltpu.VMEM((D, D), BF16),
            pltpu.VMEM((D, D), BF16),
            pltpu.VMEM((D, D), BF16),
            pltpu.VMEM((2, D, F), BF16),
            pltpu.VMEM((F, D), BF16),
            pltpu.VMEM((3 * D // 2, D), U32),
            pltpu.VMEM((3, 5, DHALF // 2, KH), U32),
            pltpu.VMEM((HB, D), U32),
            pltpu.VMEM((7, TH // 2, KH), U32),
            pltpu.VMEM((TH // 2, 256), U32),
            pltpu.VMEM((NT, D, T), U32),
            pltpu.VMEM((D, T), U32),
            pltpu.VMEM((NG, VR, PR), F32),
            pltpu.VMEM((NG, VR // 2, PR), U32),
            pltpu.VMEM((2, 49, KH // 4, FH // 2), U32),
            pltpu.VMEM((49, FH // 4, KH), U32),
            pltpu.VMEM((5, KH // 2, KH), U32),
            pltpu.VMEM((S, D), BF16),
            pltpu.SMEM((1,), U32),
            pltpu.SemaphoreType.DMA((8,)),
        ],
        compiler_params=pltpu.CompilerParams(
            vmem_limit_bytes=100 * 1024 * 1024),
        name="hedgehog_block",
    )(x, A_wqkv, wphi, A_wo, B_w_gate, B_w_up, B_w_down)
    return out.reshape(1, S, D)
```

```python
import functools
import math

import jax
import jax.numpy as jnp
from jax import lax
import jax.experimental.pallas as pl
import jax.experimental.pallas.tpu as pltpu

S, D, H, DH, F = 2048, 640, 32, 20, 1536
NG = 16
GR = 40
PR = 80
VR = 48
DHALF = D // 2
KH = 256
FH = F // 2
HB = 128
PG = 16
T = 512
NT = S // T
TH = T // 2
NW = 256
TQ = 32
KF = 3
PST = 16
KVG, KVW = 14, 2
NSH = 42
LNR, LN0, LN1 = 32, 98, 147
SA, SB = 600, 2
GORD = (0, 6, 7, 1, 8, 2, 9, 3, 10, 4, 11, 5, 12, 13, 14, 15)
LN_EPS = 1e-5
DEN_EPS = 1e-6
LOG2E = math.log2(math.e)
F32 = jnp.float32
BF16 = jnp.bfloat16
U32 = jnp.uint32


def _dot(a, b):
    return jnp.dot(a, b, preferred_element_type=F32)


def _dot_nt(a, b):
    return lax.dot_general(a, b, (((1,), (1,)), ((), ())),
                           preferred_element_type=F32)


def _pk(v):
    return pltpu.bitcast(v.astype(BF16), U32)


def _upk(w):
    return pltpu.bitcast(w, BF16)


def _hs(a, b):
    assert a % 16 == 0 and b % 16 == 0
    return slice(a // 2, b // 2)


def _layernorm(x, anchor=None):
    t = x.shape[0]
    s1 = x[:, 0:128]
    for k in range(1, D // 128):
        s1 = s1 + x[:, 128 * k:128 * (k + 1)]
    if anchor is not None:
        s1 = (s1.reshape(t // 8, 8, 128) + anchor[None]).reshape(t, 128)
    mu = jnp.sum(s1, axis=-1, keepdims=True) * (1.0 / D)
    xc = x - mu
    var = jnp.mean(xc * xc, axis=-1, keepdims=True)
    return xc * lax.rsqrt(var + LN_EPS)


def _layernorm_shifted(x, zeros=None):
    c = x[:, 0:128] if zeros is None else x[:, 0:128] + zeros
    c = c[:, 0:1]
    s1 = s2 = None
    for k in range(D // 128):
        d = x[:, 128 * k:128 * (k + 1)] - c
        s1 = d if s1 is None else s1 + d
        s2 = d * d if s2 is None else s2 + d * d
    m1 = jnp.sum(s1, axis=-1, keepdims=True) * (1.0 / D)
    m2 = jnp.sum(s2, axis=-1, keepdims=True) * (1.0 / D)
    var = jnp.maximum(m2 - m1 * m1, 0.0)
    return (x - (c + m1)) * lax.rsqrt(var + LN_EPS)


def _allred(op, t):
    t = op(t, pltpu.roll(t, 2, 1))
    return op(t, pltpu.roll(t, 4, 1))


def _recip(s):
    r = pl.reciprocal(s, approx=True)
    return r * (2.0 - s * r)


def _feature_map(p):
    n, t = p.shape[0] // GR, p.shape[1]
    p4 = p.reshape(n, 5, 8, t)
    mx = _allred(jnp.maximum, jnp.max(p4, axis=1))[:, None]
    mn = _allred(jnp.minimum, jnp.min(p4, axis=1))[:, None]
    ep = jnp.exp2(p4 - mx)
    en = jnp.exp2(mn - p4)
    sp = _allred(jnp.add, jnp.sum(ep, axis=1))[:, None]
    sn = _allred(jnp.add, jnp.sum(en, axis=1))[:, None]
    phi = jnp.concatenate([ep * _recip(sp), en * _recip(sn)], axis=1)
    return phi.reshape(n * PR, t)


def _augment_v(vt):
    n, t = vt.shape[0] // GR, vt.shape[1]
    va = jnp.concatenate([vt.reshape(n, GR, t), jnp.ones((n, 8, t), F32)], axis=1)
    return va.reshape(n * VR, t)


def _gelu(g):
    c = math.sqrt(2.0 / math.pi)
    return 0.5 * g * (1.0 + jnp.tanh(c * (g + 0.044715 * (g * g * g))))


def _lhs_sums(a11, a12, a21, a22):
    return [a11 + a22, a21 + a22, a11 + a12, a21 - a11, a12 - a22]


def _rhs_sums(b11, b12, b21, b22):
    return [b11 + b22, b12 - b22, b21 - b11, b11 + b12, b21 + b22]


def _lhs_ops(s, a11, a22):
    return [s[0], s[1], a11, a22, s[2], s[3], s[4]]


def _rhs_ops(s, b11, b22):
    return [s[0], b11, s[1], s[2], b22, s[3], s[4]]


def _strassen_steps(mm, rest, post, out):
    fin = lambda i, c: post(i, c if rest is None else c + rest[i]())
    m2 = mm(2)
    yield
    m4 = mm(4)
    yield
    out[1] = fin(1, m2 + m4)
    yield
    m3 = mm(3)
    yield
    m1 = mm(1)
    yield
    out[2] = fin(2, m3 + m1)
    yield
    m0 = mm(0)
    yield
    c11 = m3 - m4 + m0 + mm(6)
    yield
    out[0] = fin(0, c11)
    yield
    c22 = m2 - m1 + m0 + mm(5)
    yield
    out[3] = fin(3, c22)
    yield


def _run(mm, rest):
    out = [None] * 4
    for _ in _strassen_steps(mm, rest, lambda _, c: c, out):
        pass
    return out


def _quad(a):
    h, k = a.shape[0] // 2, a.shape[1] // 2
    return a[:h, :k], a[:h, k:], a[h:, :k], a[h:, k:]


def _join(c):
    return jnp.concatenate([jnp.concatenate(c[0:2], axis=1),
                            jnp.concatenate(c[2:4], axis=1)], axis=0)


def _lhs7(b):
    return _lhs_ops(_lhs_sums(*b), b[0], b[3])


def _rhs7(b):
    return _rhs_ops(_rhs_sums(*b), b[0], b[3])


def _add_tile(a, z):
    if z is None:
        return a
    r, c = a.shape
    z = jnp.concatenate([z] * (c // 128), axis=1)
    return (a.reshape(r // 8, 8, c) + z[None]).reshape(r, c)


def _lhs_row(b, i, z=None):
    a11, a12, a21, a22 = b
    if i in (2, 3):
        q = list(_quad(a11 if i == 2 else a22))
        q[0], q[3] = _add_tile(q[0], z), _add_tile(q[3], z)
        return _lhs7(q)
    x, y, sign = {0: (a11, a22, 1), 1: (a21, a22, 1), 4: (a11, a12, 1),
                  5: (a21, a11, -1), 6: (a12, a22, -1)}[i]
    x = _add_tile(x, z)
    return _lhs7(_quad(x + y if sign > 0 else x - y))


def _run_late22(mm, rest, mid):
    m2, m4 = mm(2), mm(4)
    c12 = m2 + m4 + rest[1]()
    c22 = m2 + mm(5) + rest[3]()
    mid()
    m3, m1 = mm(3), mm(1)
    c21 = m3 + m1 + rest[2]()
    m0 = mm(0)
    c22 = c22 - m1 + m0
    c11 = m3 - m4 + m0 + mm(6) + rest[0]()
    return [c11, c12, c21, c22]


def _strassen2(lhs_row, rhs, rest, mid=None, plag=3, log=None):
    seen = []

    def mm(i):
        ops = lhs_row(i, seen[-plag] if len(seen) >= plag else None)
        first = []

        def inner(j):
            m = _dot(ops[j], rhs(i, j))
            first.append(m)
            return m

        out = _join(_run(inner, None))
        seen.append(first[0][0:8, :])
        if log is not None:
            log.extend(first)
        return out

    return _run(mm, rest) if mid is None else _run_late22(mm, rest, mid)


def _chain(gens):
    for g in gens:
        yield from g


def _split_rows(a):
    n, c = a.shape
    a4 = a.reshape(n // (2 * PG), 2, PG, c)
    return a4[:, 0].reshape(n // 2, c), a4[:, 1].reshape(n // 2, c)


def _merge_rows(top, bot):
    n, c = top.shape
    both = jnp.stack([top.reshape(n // PG, PG, c), bot.reshape(n // PG, PG, c)],
                     axis=1)
    return both.reshape(2 * n, c)


def _fold_windows():
    wins = []
    for kt in range(5):
        g_lo, g_hi = (128 * kt) // GR, (128 * kt + 127) // GR
        r0 = (g_lo * GR) // 16 * 16
        r1 = -((-(g_hi + 1) * GR) // 16) * 16
        wins.append((r0, r1))
    return wins


def _kernel(x_hbm, wqkv_hbm, wphi_hbm, wo_hbm, wg_hbm, wu_hbm, wd_hbm,
            o_hbm,
            x_v, wphi_v, wk_v, wq_v, wv_v, wo_v, wgu_v, wd_v,
            wT, wS, xn0, xs, x5, phiq, phik, kvacc, kvb, sgu, sd, so, o_v,
            zero_s, sems):
    wins = _fold_windows()

    srcs = [
        (wphi_hbm, wphi_v),
        (wqkv_hbm.at[:, D:D + 128 * KF], wk_v.at[:, 0:128 * KF]),
        (x_hbm.at[0:TH], x_v.at[0:TH]),
        (wqkv_hbm.at[:, D + 128 * KF:2 * D], wk_v.at[:, 128 * KF:D]),
        (x_hbm.at[TH:T], x_v.at[TH:T]),
        (wqkv_hbm.at[:, 0:D], wq_v),
        (wqkv_hbm.at[:, 2 * D:3 * D], wv_v),
        (x_hbm.at[T:2 * T], x_v.at[T:2 * T]),
        (x_hbm.at[2 * T:S], x_v.at[2 * T:S]),
        (wg_hbm, wgu_v.at[0]),
        (wu_hbm, wgu_v.at[1]),
        (wo_hbm, wo_v),
        (wd_hbm, wd_v),
    ]
    sem_of = [0, 1, 2, 2, 3, 3, 4, 4, 5, 5, 6, 7, 7]

    def cp(k):
        return pltpu.make_async_copy(srcs[k][0], srcs[k][1], sems.at[sem_of[k]])

    def x_rows(r0, n):
        return x_v[pl.ds(pl.multiple_of(r0, 16), n), :].astype(F32)

    def fold_part(kt, bdts, w_ref):
        return _dot_nt(bdts[kt], w_ref[:, 128 * kt:128 * (kt + 1)])

    def fold_store(base, parts, kts):
        for kt in kts:
            r0, r1 = wins[kt]
            pos = r0
            pieces = []
            if kt > 0:
                p0, p1 = wins[kt - 1]
                pieces.append(parts[kt - 1][r0 - p0:] + parts[kt][:p1 - r0])
                pos = p1
            nxt = wins[kt + 1][0] if kt < 4 else r1
            pieces.append(parts[kt][pos - r0:nxt - r0])
            wT[_hs(base + r0, base + nxt), :] = _pk(
                jnp.concatenate(pieces, axis=0) * LOG2E)

    pace = []

    def note(p):
        pace.append([(p, r, n) for n in range(p.shape[1] // 128)
                     for r in range(0, p.shape[0], PST)])
        return p

    def anchors(npace, count, phase=0.0):
        pool = [tl for tiles in pace[-npace:] for tl in tiles]
        zero = zero_s[0]
        cache = {}
        out = []
        for i in range(count):
            k = int((i + phase) * len(pool) / count)
            if k not in cache:
                p, r, n = pool[k]
                tile = (p[r:r + 8, 128 * n:128 * (n + 1)] if n >= 0 else
                        jnp.broadcast_to(p[r:r + 8, 0:1], (8, 128)))
                cache[k] = pltpu.bitcast(tile, U32) & zero
            out.append(cache[k])
        return out

    def block_sums(specs, sums, npace):
        jobs = [(w, dst, rb, k2, n2, r, c)
                for w, dst, rb, k2, n2 in specs
                for r in range(0, k2, 16) for c in range(0, n2, 128)]
        ans = anchors(npace, len(jobs)) if npace else [None] * len(jobs)
        for an, (w, dst, rb, k2, n2, r, c) in zip(ans, jobs):
            def get(r0, c0, an=None):
                if w.dtype == U32:
                    bits = w[_hs(r0, r0 + 16), c0:c0 + 128]
                    return _upk(bits if an is None else bits | an).astype(F32)
                v = w[r0:r0 + 16, c0:c0 + 128].astype(F32)
                if an is None:
                    return v
                return (v.reshape(2, 8, 128)
                        + pltpu.bitcast(an, F32)[None]).reshape(16, 128)

            top, bot = rb + r, rb + k2 + r
            vals = sums(get(top, c, an), get(top, n2 + c),
                        get(bot, c), get(bot, n2 + c, an))
            for j, v in enumerate(vals):
                dst.at[j][_hs(r, r + 16), c:c + 128] = _pk(v)

    def ffn_sums_jobs(w, dst, up):
        def job(p, r, i, an):
            model = [128 * k for k in range(4)]
            ffn = [NW * p, NW * p + 128, FH + NW * p, FH + NW * p + 128]
            rws, cls = (model, ffn) if up else (ffn, model)
            z = pltpu.bitcast(an, F32)[None]

            def blk(bi, bj):
                return lambda: jnp.concatenate(
                    [w[rws[2 * bi + k] + r:rws[2 * bi + k] + r + 16,
                       cls[2 * bj]:cls[2 * bj] + 256].astype(F32)
                     for k in range(2)], axis=0)

            b11, b12, b21, b22 = blk(0, 0), blk(0, 1), blk(1, 0), blk(1, 1)
            op = [lambda: b11() + b22(), b11, lambda: b12() - b22(),
                  lambda: b21() - b11(), b22, lambda: b11() + b12(),
                  lambda: b21() + b22()][i]()
            q = list(_quad(op))
            for k in (0, 3):
                q[k] = (q[k].reshape(2, 8, 128) + z).reshape(16, 128)
            r0, c0 = (r, 128 * p) if up else (128 * p + r, 0)
            for j, v in enumerate(_rhs7(q)):
                dst.at[7 * i + j][_hs(r0, r0 + 16), c0:c0 + 128] = _pk(v)

        return [functools.partial(job, p, r, i) for p in range(FH // NW)
                for r in range(0, 128, 16) for i in range(7)]

    def run_jobs(jobs, npace):
        for an, job in zip(anchors(npace, len(jobs), 0.5), jobs):
            job(an)

    def ln_pair(i, r0, anchor=None):
        xn = _layernorm(x_rows(r0, 2 * PG), anchor)
        lo, hi = xn[:PG], xn[PG:]
        b11, b12 = lo[:, 0:KH], hi[:, 0:KH]
        b21, b22 = lo[:, KH:2 * KH], hi[:, KH:2 * KH]
        rows = _hs(PG * i, PG * (i + 1))
        for j, v in enumerate(_rhs_ops(_rhs_sums(b11, b12, b21, b22), b11, b22)):
            xs.at[j][rows, :] = _pk(v)
        x5[rows, :] = _pk(jnp.concatenate([lo[:, 2 * KH:], hi[:, 2 * KH:]], axis=1))
        return lo, hi

    def ln_next(t, npace):
        for i, an in enumerate(anchors(npace, T // (2 * PG))):
            ln_pair(i, t * T + 2 * PG * i, pltpu.bitcast(an, F32))

    def proj_steps(m, n, post, out):
        top = _hs(m * D, m * D + DHALF)
        bot = _hs(m * D + DHALF, (m + 1) * D)
        tok = _hs(HB * n, HB * (n + 1))
        lhs = _lhs_ops([lambda j=j: wS[m, j] for j in range(5)],
                       lambda: wT[top, 0:KH], lambda: wT[bot, KH:2 * KH])
        rest = [lambda r=r, c=c: _dot_nt(_upk(wT[r, 2 * KH:D]),
                                         _upk(x5[tok, 128 * c:128 * (c + 1)]))
                for r in (top, bot) for c in range(2)]
        return _strassen_steps(
            lambda i: note(_dot_nt(_upk(lhs[i]()), _upk(xs[i, tok, :]))),
            rest, post, out)

    def kv_update(vta, last):
        if last:
            row = lax.broadcasted_iota(jnp.int32, (VR, PR), 0)
            odd = lax.broadcasted_iota(jnp.int32, (VR, PR), 1) & 1
            second = jnp.logical_or(
                jnp.logical_and(row >= DH, row < GR), row >= GR + 4)
            keep = odd == second.astype(jnp.int32)
        for g in range(NG):
            c, gg = divmod(g, 8)
            upd = _dot_nt(vta[c][gg * VR:(gg + 1) * VR, :].astype(BF16),
                          _upk(phik[_hs(g * PR, (g + 1) * PR), :]))
            if g < KVG:
                pace.append([(upd, r, -1) for r in range(0, VR, 8)
                             for _ in range(KVW)])
            if last:
                kvb.at[g][...] = _pk(jnp.where(keep, kvacc[g] + upd, 0.0))
            else:
                kvacc[g] += upd

    def w_sums(m, npace):
        block_sums([(wT, wS.at[m], m * D, DHALF, KH)], _lhs_sums, npace)

    pending = []

    def store_phi(dst, n):
        def post(i, c):
            r, hi = divmod(i, 2)
            pending.append((dst, r, TH * hi + HB * n, _feature_map(c)))
        return post

    def flush(which=None):
        keep = []
        for dst, r, l0, phi in pending:
            if which is None or dst is which:
                dst[_hs(D * r, D * (r + 1)), l0:l0 + HB] = _pk(phi)
            else:
                keep.append((dst, r, l0, phi))
        pending[:] = keep

    def p1_run(t, mains, voff, every, skip, extra, last, late=None):
        nb = TH // HB
        vout = [[None] * 4 for _ in range(nb)]
        dsts = [phik, phiq.at[t]]
        n0 = len(pace)
        main = _chain([proj_steps(m, n, store_phi(dsts[m], n), [None] * 4)
                       for m, n in mains])
        side = _chain([proj_steps(2, n, lambda i, c: _augment_v(c), vout[n])
                       for n in range(nb)])
        for i, _ in enumerate(main):
            if i + 1 >= voff and i % every == every - 1:
                next(side, None)
        for _ in side:
            pass
        flush(dsts[1])
        extra(len(pace) - n0 - skip)
        flush()
        kv_update([jnp.concatenate([vout[n][2 * r + hi] for hi in range(2)
                                    for n in range(nb)], axis=1)
                   for r in range(2)], last)
        if late is not None:
            late(len(pace) - n0)

    for k in range(len(srcs)):
        cp(k).start()
    zero_s[0] = jnp.uint32(0)
    kvacc[...] = jnp.zeros(kvacc.shape, F32)
    rel = (lax.broadcasted_iota(jnp.int32, (H, D), 1)
           - DH * lax.broadcasted_iota(jnp.int32, (H, D), 0))
    e2 = jnp.where(
        lax.broadcasted_iota(jnp.int32, (VR, DH), 0) >> 1
        == lax.broadcasted_iota(jnp.int32, (VR, DH), 1), 1.0, 0.0).astype(BF16)
    lane8 = lax.broadcasted_iota(jnp.int32, (8, 128), 1)
    sub8 = lax.broadcasted_iota(jnp.int32, (8, 128), 0)
    cp(0).wait()
    m = None
    for d in range(DH):
        sel = jnp.where(rel == d, 1.0, 0.0).astype(BF16)
        t = _dot(wphi_v[d], sel)
        m = t if m is None else m + t
    m2 = _dot(e2, m.astype(BF16))[0:GR]
    relp = lane8 - DH * (sub8 & 1)
    bdts = []
    for kt in range(5):
        r0, r1 = wins[kt]
        pat = m2[:, 128 * kt:128 * (kt + 1)].reshape(5, 8, 128)
        rows = []
        r = r0
        while r < r1:
            g, o = divmod(r, GR)
            n = min(GR - o, r1 - r)
            c0 = GR * g - 128 * kt
            msk = jnp.logical_and(relp >= c0, relp < c0 + DH)
            rows.append(jnp.where(msk[None], pat[o // 8:(o + n) // 8], 0.0))
            r += n
        bdts.append(jnp.concatenate(rows, axis=0)
                    .reshape(r1 - r0, 128).astype(BF16))

    cp(1).wait()
    parts = [fold_part(kt, bdts, wk_v) for kt in range(KF)]
    fold_store(0, parts, range(KF))
    cp(2).wait()
    cp(3).wait()
    for i in range(HB // PG):
        lo, hi = ln_pair(i, 2 * PG * i)
        xn0[_hs(PG * i, PG * (i + 1)), :] = _pk(lo)
        xn0[_hs(HB + PG * i, HB + PG * (i + 1)), :] = _pk(hi)
    parts += [fold_part(kt, bdts, wk_v) for kt in range(KF, 5)]
    fold_store(0, parts, range(KF, 5))
    for r in range(2):
        phi = _feature_map(note(_dot_nt(
            _upk(wT[_hs(DHALF * r, DHALF * (r + 1)), :]), _upk(xn0[...]))))
        for hi in range(2):
            phik[_hs(D * r, D * (r + 1)), TH * hi:TH * hi + HB] = _pk(
                phi[:, HB * hi:HB * (hi + 1)])
    w_sums(0, 2)
    cp(4).wait()
    cp(5).wait()
    for i in range(HB // PG, TH // PG):
        ln_pair(i, 2 * PG * i)
    fold_store(D, [fold_part(kt, bdts, wq_v) for kt in range(5)], range(5))
    for _ in proj_steps(0, 1, store_phi(phik, 1), [None] * 4):
        pass
    flush()
    w_sums(1, 7)
    cp(6).wait()
    cp(7).wait()
    wT[_hs(2 * D, 3 * D), :] = _pk(wv_v[...].T)
    w_sums(2, 0)
    p1_run(0, ((1, 0), (1, 1)), 8, 1, 10, lambda n: ln_next(1, n), False)
    cp(8).wait()
    cp(9).wait()

    all_mains = ((0, 0), (0, 1), (1, 0), (1, 1))

    def p1_body(t, carry):
        @pl.when(t == 2)
        def _():
            cp(10).wait()

        p1_run(t, all_mains, 12, 2, 0, lambda n: ln_next(t + 1, n), False,
               lambda n: run_jobs(
                   ffn_sums_jobs(wgu_v.at[t - 1], sgu.at[t - 1], True)[NSH:], n))
        return carry

    lax.fori_loop(1, NT - 1, p1_body, 0)
    cp(11).wait()
    cp(12).wait()

    p1_run(NT - 1, all_mains, 12, 2, 0,
           lambda n: block_sums([(wo_v, so, 0, KH, KH)], _rhs_sums, n), True,
           lambda n: run_jobs(
               ffn_sums_jobs(wgu_v.at[0], sgu.at[0], True)[:NSH]
               + ffn_sums_jobs(wgu_v.at[1], sgu.at[1], True)[:NSH]
               + ffn_sums_jobs(wd_v, sd, False), n))

    def att_num(ti, b):
        def phi(g):
            rows = _hs(PR * g, PR * (g + 1))
            return _upk(jnp.concatenate(
                [phiq[ti, rows, c0:c0 + HB] for c0 in (HB * b, TH + HB * b)],
                axis=1))

        gnum = [None] * NG
        for g in GORD:
            gnum[g] = _dot(_upk(kvb[g]), phi(g))
        sub = lax.broadcasted_iota(jnp.int32, (8, 2 * HB), 0) < 4
        pieces = []
        for g in range(NG):
            rec = _recip(gnum[g][GR:VR] + DEN_EPS)
            rot = pltpu.roll(rec, 4, 0)
            ra = jnp.where(sub, rec, rot)
            rb = jnp.where(sub, rot, rec)
            scale = jnp.concatenate([ra, ra, rec, rb, rb], axis=0)
            pieces.append(gnum[g][0:GR] * scale)
        return jnp.concatenate(pieces, axis=0)

    def zero_of(tile):
        if tile is None:
            return None
        return pltpu.bitcast(pltpu.bitcast(tile, U32) & zero_s[0], F32)

    def att_sums(ot, z):
        sums = _lhs_sums(_add_tile(ot[0:KH, :HB], z), ot[KH:2 * KH, :HB],
                         ot[0:KH, HB:], _add_tile(ot[KH:2 * KH, HB:], z))
        st = jnp.concatenate(
            [jnp.concatenate([v[:128], v[128:]], axis=1) for v in sums], axis=0)
        st = st.astype(BF16).T
        return [jnp.concatenate([st[:HB, 128 * j:128 * (j + 1)],
                                 st[HB:, 128 * j:128 * (j + 1)]], axis=1)
                for j in range(5)]

    def att_out(ti, b, ot, tile):
        xt, xb = _split_rows(x_rows(ti * T + 2 * HB * b, 2 * HB))
        o = ot.astype(BF16).T
        c5 = _dot(o, wo_v[:, 2 * KH:D])
        r5 = _dot(o[:, 2 * KH:], wo_v[2 * KH:D, 0:2 * KH])
        sums = att_sums(ot, zero_of(tile))
        lhs = _lhs_ops(sums, o[:HB, 0:KH], o[HB:, KH:2 * KH])
        rhs = _rhs_ops([_upk(so[j]) for j in range(5)],
                       wo_v[0:KH, 0:KH], wo_v[KH:2 * KH, KH:2 * KH])
        mm = lambda i: _dot(lhs[i], rhs[i])
        m2, m3, m4, m0 = mm(2), mm(3), mm(4), mm(0)
        c12 = m2 + m4 + r5[:HB, KH:]
        c11 = m3 - m4 + m0 + mm(6) + r5[:HB, :KH]
        ht = xt + jnp.concatenate([c11, c12, c5[:HB]], axis=1)
        m1 = mm(1)
        c21 = m3 + m1 + r5[HB:, :KH]
        c22 = m2 - m1 + m0 + mm(5) + r5[HB:, KH:]
        hb = xb + jnp.concatenate([c21, c22, c5[HB:]], axis=1)
        return (ht, hb), [c5, r5, m2, m3, m4, m0, m1]

    def out_cp(r0, n):
        rows = pl.ds(pl.multiple_of(r0, 16), n)
        return pltpu.make_async_copy(o_v.at[rows], o_hbm.at[rows], sems.at[0])

    class Ffn:
        def __init__(self, base, halves, tq, tiles=None):
            ht, hb = halves
            zs = [None, None]
            if tiles is not None:
                n = HB // LNR
                pick = [zero_of(tiles[k * len(tiles) // n][0:8, :]) for k in range(n)]
                zs = [jnp.concatenate([z for z in pick for _ in range(LNR // 8)],
                                      axis=0)] * 2
            nt_, nb = _layernorm_shifted(ht, zs[0]), _layernorm_shifted(hb, zs[1])
            self.log = []
            self.base, self.tq = base, tq
            self.hn = (nt_[:, 0:KH], nt_[:, KH:2 * KH], nb[:, 0:KH], nb[:, KH:2 * KH])
            self.lhs = {}
            self.a5 = [nt_[:, 2 * KH:].astype(BF16), nb[:, 2 * KH:].astype(BF16)]
            self.cs = [ht[:, 0:KH], ht[:, KH:2 * KH], hb[:, 0:KH], hb[:, KH:2 * KH]]
            self.c5 = jnp.concatenate([ht[:, 2 * KH:], hb[:, 2 * KH:]], axis=0)
            self.act = {}

        def up(self, p):
            cols = (slice(NW * p, NW * (p + 1)), slice(FH + NW * p, FH + NW * (p + 1)))

            def proj(m):
                rest = [functools.partial(_dot, a, wgu_v[m, 2 * KH:D, c])
                        for a in self.a5 for c in cols]

                def lhs_row(i, tile):
                    if i not in self.lhs:
                        self.lhs[i] = [v.astype(BF16) for v in
                                       _lhs_row(self.hn, i, zero_of(tile))]
                    return self.lhs[i]

                return _strassen2(
                    lhs_row,
                    lambda i, j: _upk(sgu[m, 7 * i + j, :, 128 * p:128 * (p + 1)]),
                    rest, log=self.log)

            g, u = proj(0), proj(1)
            self.act[p] = [_gelu(g[i]) * u[i] for i in range(4)]

        def down(self, p):
            act = self.act.pop(p)

            def last_tile(k):
                a = jnp.concatenate([act[k], act[2 + k]], axis=0).astype(BF16)
                r0 = FH * k + NW * p
                self.c5 = self.c5 + _dot(a, wd_v[r0:r0 + NW, 2 * KH:D])

            last_tile(0)
            rhs = lambda i, j: _upk(sd[7 * i + j, _hs(128 * p, 128 * (p + 1)), 0:128])
            if p < FH // NW - 1:
                self.cs = _strassen2(
                    lambda i, tile: [v.astype(BF16) for v in
                                     _lhs_row(act, i, zero_of(tile))],
                    rhs, [lambda c=c: c for c in self.cs], lambda: last_tile(1))
                return
            tq, hq = self.tq, HB // 2
            for q in range(0, hq, tq):
                pick = lambda c: jnp.concatenate(
                    [c[q:q + tq], c[hq + q:hq + q + tq]], axis=0)
                sub = [pick(a) for a in act]
                f = _strassen2(lambda i, tile: [v.astype(BF16) for v in
                                                _lhs_row(sub, i, zero_of(tile))],
                               rhs,
                               [lambda c=c: pick(c) for c in self.cs],
                               lambda: last_tile(1) if q == 0 else None,
                               plag=3 * hq // tq)
                top = jnp.concatenate([f[0], f[1], pick(self.c5[:HB])], axis=1)
                bot = jnp.concatenate([f[2], f[3], pick(self.c5[HB:])], axis=1)
                for k in range(2):
                    res = _merge_rows(top[tq * k:tq * (k + 1)], bot[tq * k:tq * (k + 1)])
                    r0 = self.base + 2 * (hq * k + q)
                    o_v[pl.ds(pl.multiple_of(r0, 2 * tq), 2 * tq), :] = res.astype(BF16)
                    out_cp(r0, 2 * tq).start()

    def p2_body(t, carry):
        nb = TH // HB
        ots = [att_num(t, b) for b in range(nb)]
        hs = []
        tile = ots[1][SA:SA + 8, 0:128]
        for b in range(nb):
            h, res = att_out(t, b, ots[b], tile)
            hs.append(h)
            tile = res[SB][0:8, 0:128]
        tiles = None
        for b in range(nb):
            f = Ffn(t * T + 2 * HB * b, hs[b], TQ if b + 1 == nb else HB // 2, tiles)
            for p in range(FH // NW):
                f.up(p)
                f.down(p)
            tiles = f.log[LN0:LN1]
        return carry

    lax.fori_loop(0, NT, p2_body, 0)
    pltpu.make_async_copy(o_v, o_hbm, sems.at[0]).wait()


@jax.jit
def pallas_sequential_preLN__linear_kernel_hedgehog__geglu_ffn__prompt_kernel(
    A_x: jax.Array,
    A_wqkv: jax.Array,
    A_w_phi: jax.Array,
    A_wo: jax.Array,
    B_x: jax.Array,
    B_w_gate: jax.Array,
    B_w_up: jax.Array,
    B_w_down: jax.Array,
):
    del B_x
    x = A_x.reshape(S, D)
    wphi = jnp.transpose(A_w_phi, (1, 2, 0))
    any_spec = pl.BlockSpec(memory_space=pl.ANY)
    out = pl.pallas_call(
        _kernel,
        in_specs=[any_spec] * 7,
        out_specs=any_spec,
        out_shape=jax.ShapeDtypeStruct((S, D), BF16),
        scratch_shapes=[
            pltpu.VMEM((S, D), BF16),
            pltpu.VMEM((DH, DH, H), BF16),
            pltpu.VMEM((D, D), BF16),
            pltpu.VMEM((D, D), BF16),
            pltpu.VMEM((D, D), BF16),
            pltpu.VMEM((D, D), BF16),
            pltpu.VMEM((2, D, F), BF16),
            pltpu.VMEM((F, D), BF16),
            pltpu.VMEM((3 * D // 2, D), U32),
            pltpu.VMEM((3, 5, DHALF // 2, KH), U32),
            pltpu.VMEM((HB, D), U32),
            pltpu.VMEM((7, TH // 2, KH), U32),
            pltpu.VMEM((TH // 2, 256), U32),
            pltpu.VMEM((NT, D, T), U32),
            pltpu.VMEM((D, T), U32),
            pltpu.VMEM((NG, VR, PR), F32),
            pltpu.VMEM((NG, VR // 2, PR), U32),
            pltpu.VMEM((2, 49, KH // 4, FH // 2), U32),
            pltpu.VMEM((49, FH // 4, KH), U32),
            pltpu.VMEM((5, KH // 2, KH), U32),
            pltpu.VMEM((S, D), BF16),
            pltpu.SMEM((1,), U32),
            pltpu.SemaphoreType.DMA((8,)),
        ],
        compiler_params=pltpu.CompilerParams(
            vmem_limit_bytes=100 * 1024 * 1024),
        name="hedgehog_block",
    )(x, A_wqkv, wphi, A_wo, B_w_gate, B_w_up, B_w_down)
    return out.reshape(1, S, D)
```

```python
import functools
import math

import jax
import jax.numpy as jnp
from jax import lax
import jax.experimental.pallas as pl
import jax.experimental.pallas.tpu as pltpu

S, D, H, DH, F = 2048, 640, 32, 20, 1536
NG = 16
GR = 40
PR = 80
VR = 48
DHALF = D // 2
KH = 256
FH = F // 2
HB = 128
PG = 16
T = 512
NT = S // T
TH = T // 2
NW = 256
TQ = 32
KF = 3
PST = 16
KVG, KVW = 14, 2
NSH = 42
LNR, LN0, LN1 = 32, 98, 147
SWAP = (0, 1, 2)
SA, SB = 600, 2
GORD = (0, 6, 7, 1, 8, 2, 9, 3, 10, 4, 11, 5, 12, 13, 14, 15)
LN_EPS = 1e-5
DEN_EPS = 1e-6
LOG2E = math.log2(math.e)
F32 = jnp.float32
BF16 = jnp.bfloat16
U32 = jnp.uint32


def _dot(a, b):
    return jnp.dot(a, b, preferred_element_type=F32)


def _dot_nt(a, b):
    return lax.dot_general(a, b, (((1,), (1,)), ((), ())),
                           preferred_element_type=F32)


def _pk(v):
    return pltpu.bitcast(v.astype(BF16), U32)


def _upk(w):
    return pltpu.bitcast(w, BF16)


def _hs(a, b):
    assert a % 16 == 0 and b % 16 == 0
    return slice(a // 2, b // 2)


def _layernorm(x, anchor=None):
    t = x.shape[0]
    s1 = x[:, 0:128]
    for k in range(1, D // 128):
        s1 = s1 + x[:, 128 * k:128 * (k + 1)]
    if anchor is not None:
        s1 = (s1.reshape(t // 8, 8, 128) + anchor[None]).reshape(t, 128)
    mu = jnp.sum(s1, axis=-1, keepdims=True) * (1.0 / D)
    xc = x - mu
    var = jnp.mean(xc * xc, axis=-1, keepdims=True)
    return xc * lax.rsqrt(var + LN_EPS)


def _layernorm_shifted(x, zeros=None):
    c = x[:, 0:128] if zeros is None else x[:, 0:128] + zeros
    c = c[:, 0:1]
    s1 = s2 = None
    for k in range(D // 128):
        d = x[:, 128 * k:128 * (k + 1)] - c
        s1 = d if s1 is None else s1 + d
        s2 = d * d if s2 is None else s2 + d * d
    m1 = jnp.sum(s1, axis=-1, keepdims=True) * (1.0 / D)
    m2 = jnp.sum(s2, axis=-1, keepdims=True) * (1.0 / D)
    var = jnp.maximum(m2 - m1 * m1, 0.0)
    return (x - (c + m1)) * lax.rsqrt(var + LN_EPS)


def _allred(op, t):
    t = op(t, pltpu.roll(t, 2, 1))
    return op(t, pltpu.roll(t, 4, 1))


def _recip(s):
    r = pl.reciprocal(s, approx=True)
    return r * (2.0 - s * r)


def _feature_map(p):
    n, t = p.shape[0] // GR, p.shape[1]
    p4 = p.reshape(n, 5, 8, t)
    mx = _allred(jnp.maximum, jnp.max(p4, axis=1))[:, None]
    mn = _allred(jnp.minimum, jnp.min(p4, axis=1))[:, None]
    ep = jnp.exp2(p4 - mx)
    en = jnp.exp2(mn - p4)
    sp = _allred(jnp.add, jnp.sum(ep, axis=1))[:, None]
    sn = _allred(jnp.add, jnp.sum(en, axis=1))[:, None]
    phi = jnp.concatenate([ep * _recip(sp), en * _recip(sn)], axis=1)
    return phi.reshape(n * PR, t)


def _augment_v(vt):
    n, t = vt.shape[0] // GR, vt.shape[1]
    va = jnp.concatenate([vt.reshape(n, GR, t), jnp.ones((n, 8, t), F32)], axis=1)
    return va.reshape(n * VR, t)


def _gelu(g):
    c = math.sqrt(2.0 / math.pi)
    return 0.5 * g * (1.0 + jnp.tanh(c * (g + 0.044715 * (g * g * g))))


def _lhs_sums(a11, a12, a21, a22):
    return [a11 + a22, a21 + a22, a11 + a12, a21 - a11, a12 - a22]


def _rhs_sums(b11, b12, b21, b22):
    return [b11 + b22, b12 - b22, b21 - b11, b11 + b12, b21 + b22]


def _lhs_ops(s, a11, a22):
    return [s[0], s[1], a11, a22, s[2], s[3], s[4]]


def _rhs_ops(s, b11, b22):
    return [s[0], b11, s[1], s[2], b22, s[3], s[4]]


def _strassen_steps(mm, rest, post, out):
    fin = lambda i, c: post(i, c if rest is None else c + rest[i]())
    m2 = mm(2)
    yield
    m4 = mm(4)
    yield
    out[1] = fin(1, m2 + m4)
    yield
    m3 = mm(3)
    yield
    m1 = mm(1)
    yield
    out[2] = fin(2, m3 + m1)
    yield
    m0 = mm(0)
    yield
    c11 = m3 - m4 + m0 + mm(6)
    yield
    out[0] = fin(0, c11)
    yield
    c22 = m2 - m1 + m0 + mm(5)
    yield
    out[3] = fin(3, c22)
    yield


def _run(mm, rest):
    out = [None] * 4
    for _ in _strassen_steps(mm, rest, lambda _, c: c, out):
        pass
    return out


def _quad(a):
    h, k = a.shape[0] // 2, a.shape[1] // 2
    return a[:h, :k], a[:h, k:], a[h:, :k], a[h:, k:]


def _join(c):
    return jnp.concatenate([jnp.concatenate(c[0:2], axis=1),
                            jnp.concatenate(c[2:4], axis=1)], axis=0)


def _lhs7(b):
    return _lhs_ops(_lhs_sums(*b), b[0], b[3])


def _rhs7(b):
    return _rhs_ops(_rhs_sums(*b), b[0], b[3])


def _add_tile(a, z):
    if z is None:
        return a
    r, c = a.shape
    z = jnp.concatenate([z] * (c // 128), axis=1)
    return (a.reshape(r // 8, 8, c) + z[None]).reshape(r, c)


def _lhs_row(b, i, z=None):
    a11, a12, a21, a22 = b
    if i in (2, 3):
        q = list(_quad(a11 if i == 2 else a22))
        q[0], q[3] = _add_tile(q[0], z), _add_tile(q[3], z)
        return _lhs7(q)
    x, y, sign = {0: (a11, a22, 1), 1: (a21, a22, 1), 4: (a11, a12, 1),
                  5: (a21, a11, -1), 6: (a12, a22, -1)}[i]
    x = _add_tile(x, z)
    return _lhs7(_quad(x + y if sign > 0 else x - y))


_USES = {0: ((0, 1), (3, 1)), 1: ((2, 1), (3, -1)), 2: ((1, 1), (3, 1)),
         3: ((0, 1), (2, 1)), 4: ((0, -1), (1, 1)), 5: ((3, 1),), 6: ((0, 1),)}


def _run_order(mm, cs, order, mid):
    cs = list(cs)
    for i in order:
        if i is None:
            mid()
            continue
        m = mm(i)
        for k, sign in _USES[i]:
            cs[k] = cs[k] + m if sign > 0 else cs[k] - m
    return cs


def _strassen2(lhs_row, rhs, rest, order=None, mid=None, plag=3, log=None):
    seen = []

    def mm(i):
        ops = lhs_row(i, seen[-plag] if len(seen) >= plag else None)
        first = []

        def inner(j):
            m = _dot(ops[j], rhs(i, j))
            first.append(m)
            return m

        out = _join(_run(inner, None))
        seen.append(first[0][0:8, :])
        if log is not None:
            log.extend(first)
        return out

    return _run(mm, rest) if order is None else _run_order(mm, rest, order, mid)


def _chain(gens):
    for g in gens:
        yield from g


def _split_rows(a):
    n, c = a.shape
    a4 = a.reshape(n // (2 * PG), 2, PG, c)
    return a4[:, 0].reshape(n // 2, c), a4[:, 1].reshape(n // 2, c)


def _merge_rows(top, bot):
    n, c = top.shape
    both = jnp.stack([top.reshape(n // PG, PG, c), bot.reshape(n // PG, PG, c)],
                     axis=1)
    return both.reshape(2 * n, c)


def _fold_windows():
    wins = []
    for kt in range(5):
        g_lo, g_hi = (128 * kt) // GR, (128 * kt + 127) // GR
        r0 = (g_lo * GR) // 16 * 16
        r1 = -((-(g_hi + 1) * GR) // 16) * 16
        wins.append((r0, r1))
    return wins


def _kernel(x_hbm, wqkv_hbm, wphi_hbm, wo_hbm, wg_hbm, wu_hbm, wd_hbm,
            o_hbm,
            x_v, wphi_v, wk_v, wq_v, wv_v, wo_v, wgu_v, wd_v,
            wT, wS, xn0, xs, x5, phiq, phik, kvacc, kvb, sgu, sd, so, o_v,
            zero_s, sems):
    wins = _fold_windows()

    srcs = [
        (wphi_hbm, wphi_v),
        (wqkv_hbm.at[:, D:D + 128 * KF], wk_v.at[:, 0:128 * KF]),
        (x_hbm.at[0:TH], x_v.at[0:TH]),
        (wqkv_hbm.at[:, D + 128 * KF:2 * D], wk_v.at[:, 128 * KF:D]),
        (x_hbm.at[TH:T], x_v.at[TH:T]),
        (wqkv_hbm.at[:, 0:D], wq_v),
        (wqkv_hbm.at[:, 2 * D:3 * D], wv_v),
        (x_hbm.at[T:2 * T], x_v.at[T:2 * T]),
        (x_hbm.at[2 * T:S], x_v.at[2 * T:S]),
        (wg_hbm, wgu_v.at[0]),
        (wu_hbm, wgu_v.at[1]),
        (wo_hbm, wo_v),
        (wd_hbm, wd_v),
    ]
    sem_of = [0, 1, 2, 2, 3, 3, 4, 4, 5, 5, 6, 7, 7]

    def cp(k):
        return pltpu.make_async_copy(srcs[k][0], srcs[k][1], sems.at[sem_of[k]])

    def x_rows(r0, n):
        return x_v[pl.ds(pl.multiple_of(r0, 16), n), :].astype(F32)

    def fold_part(kt, bdts, w_ref):
        return _dot_nt(bdts[kt], w_ref[:, 128 * kt:128 * (kt + 1)])

    def fold_store(base, parts, kts):
        for kt in kts:
            r0, r1 = wins[kt]
            pos = r0
            pieces = []
            if kt > 0:
                p0, p1 = wins[kt - 1]
                pieces.append(parts[kt - 1][r0 - p0:] + parts[kt][:p1 - r0])
                pos = p1
            nxt = wins[kt + 1][0] if kt < 4 else r1
            pieces.append(parts[kt][pos - r0:nxt - r0])
            wT[_hs(base + r0, base + nxt), :] = _pk(
                jnp.concatenate(pieces, axis=0) * LOG2E)

    pace = []

    def note(p):
        pace.append([(p, r, n) for n in range(p.shape[1] // 128)
                     for r in range(0, p.shape[0], PST)])
        return p

    def anchors(npace, count, phase=0.0):
        pool = [tl for tiles in pace[-npace:] for tl in tiles]
        zero = zero_s[0]
        cache = {}
        out = []
        for i in range(count):
            k = int((i + phase) * len(pool) / count)
            if k not in cache:
                p, r, n = pool[k]
                tile = (p[r:r + 8, 128 * n:128 * (n + 1)] if n >= 0 else
                        jnp.broadcast_to(p[r:r + 8, 0:1], (8, 128)))
                cache[k] = pltpu.bitcast(tile, U32) & zero
            out.append(cache[k])
        return out

    def block_sums(specs, sums, npace):
        jobs = [(w, dst, rb, k2, n2, r, c)
                for w, dst, rb, k2, n2 in specs
                for r in range(0, k2, 16) for c in range(0, n2, 128)]
        ans = anchors(npace, len(jobs)) if npace else [None] * len(jobs)
        for an, (w, dst, rb, k2, n2, r, c) in zip(ans, jobs):
            def get(r0, c0, an=None):
                if w.dtype == U32:
                    bits = w[_hs(r0, r0 + 16), c0:c0 + 128]
                    return _upk(bits if an is None else bits | an).astype(F32)
                v = w[r0:r0 + 16, c0:c0 + 128].astype(F32)
                if an is None:
                    return v
                return (v.reshape(2, 8, 128)
                        + pltpu.bitcast(an, F32)[None]).reshape(16, 128)

            top, bot = rb + r, rb + k2 + r
            vals = sums(get(top, c, an), get(top, n2 + c),
                        get(bot, c), get(bot, n2 + c, an))
            for j, v in enumerate(vals):
                dst.at[j][_hs(r, r + 16), c:c + 128] = _pk(v)

    def ffn_sums_jobs(w, dst, up):
        def job(p, r, i, an):
            model = [128 * k for k in range(4)]
            ffn = [NW * p, NW * p + 128, FH + NW * p, FH + NW * p + 128]
            rws, cls = (model, ffn) if up else (ffn, model)
            z = pltpu.bitcast(an, F32)[None]

            def blk(bi, bj):
                return lambda: jnp.concatenate(
                    [w[rws[2 * bi + k] + r:rws[2 * bi + k] + r + 16,
                       cls[2 * bj]:cls[2 * bj] + 256].astype(F32)
                     for k in range(2)], axis=0)

            b11, b12, b21, b22 = blk(0, 0), blk(0, 1), blk(1, 0), blk(1, 1)
            op = [lambda: b11() + b22(), b11, lambda: b12() - b22(),
                  lambda: b21() - b11(), b22, lambda: b11() + b12(),
                  lambda: b21() + b22()][i]()
            q = list(_quad(op))
            for k in (0, 3):
                q[k] = (q[k].reshape(2, 8, 128) + z).reshape(16, 128)
            r0, c0 = (r, 128 * p) if up else (128 * p + r, 0)
            for j, v in enumerate(_rhs7(q)):
                dst.at[7 * i + j][_hs(r0, r0 + 16), c0:c0 + 128] = _pk(v)

        return [functools.partial(job, p, r, i) for p in range(FH // NW)
                for r in range(0, 128, 16) for i in range(7)]

    def run_jobs(jobs, npace):
        for an, job in zip(anchors(npace, len(jobs), 0.5), jobs):
            job(an)

    def ln_pair(i, r0, anchor=None):
        xn = _layernorm(x_rows(r0, 2 * PG), anchor)
        lo, hi = xn[:PG], xn[PG:]
        b11, b12 = lo[:, 0:KH], hi[:, 0:KH]
        b21, b22 = lo[:, KH:2 * KH], hi[:, KH:2 * KH]
        rows = _hs(PG * i, PG * (i + 1))
        for j, v in enumerate(_rhs_ops(_rhs_sums(b11, b12, b21, b22), b11, b22)):
            xs.at[j][rows, :] = _pk(v)
        x5[rows, :] = _pk(jnp.concatenate([lo[:, 2 * KH:], hi[:, 2 * KH:]], axis=1))
        return lo, hi

    def ln_next(t, npace):
        for i, an in enumerate(anchors(npace, T // (2 * PG))):
            ln_pair(i, t * T + 2 * PG * i, pltpu.bitcast(an, F32))

    def proj_steps(m, n, post, out):
        top = _hs(m * D, m * D + DHALF)
        bot = _hs(m * D + DHALF, (m + 1) * D)
        tok = _hs(HB * n, HB * (n + 1))
        lhs = _lhs_ops([lambda j=j: wS[m, j] for j in range(5)],
                       lambda: wT[top, 0:KH], lambda: wT[bot, KH:2 * KH])
        rest = [lambda r=r, c=c: _dot_nt(_upk(wT[r, 2 * KH:D]),
                                         _upk(x5[tok, 128 * c:128 * (c + 1)]))
                for r in (top, bot) for c in range(2)]
        return _strassen_steps(
            lambda i: note(_dot_nt(_upk(lhs[i]()), _upk(xs[i, tok, :]))),
            rest, post, out)

    def kv_update(vta, last):
        if last:
            row = lax.broadcasted_iota(jnp.int32, (VR, PR), 0)
            odd = lax.broadcasted_iota(jnp.int32, (VR, PR), 1) & 1
            second = jnp.logical_or(
                jnp.logical_and(row >= DH, row < GR), row >= GR + 4)
            keep = odd == second.astype(jnp.int32)
        for g in range(NG):
            c, gg = divmod(g, 8)
            upd = _dot_nt(vta[c][gg * VR:(gg + 1) * VR, :].astype(BF16),
                          _upk(phik[_hs(g * PR, (g + 1) * PR), :]))
            if g < KVG:
                pace.append([(upd, r, -1) for r in range(0, VR, 8)
                             for _ in range(KVW)])
            if last:
                kvb.at[g][...] = _pk(jnp.where(keep, kvacc[g] + upd, 0.0))
            else:
                kvacc[g] += upd

    def w_sums(m, npace):
        block_sums([(wT, wS.at[m], m * D, DHALF, KH)], _lhs_sums, npace)

    pending = []

    def store_phi(dst, n):
        def post(i, c):
            r, hi = divmod(i, 2)
            pending.append((dst, r, TH * hi + HB * n, _feature_map(c)))
        return post

    def flush(which=None):
        keep = []
        for dst, r, l0, phi in pending:
            if which is None or dst is which:
                dst[_hs(D * r, D * (r + 1)), l0:l0 + HB] = _pk(phi)
            else:
                keep.append((dst, r, l0, phi))
        pending[:] = keep

    def p1_run(t, mains, voff, every, skip, extra, last, late=None):
        nb = TH // HB
        vout = [[None] * 4 for _ in range(nb)]
        dsts = [phik, phiq.at[t]]
        n0 = len(pace)
        main = _chain([proj_steps(m, n, store_phi(dsts[m], n), [None] * 4)
                       for m, n in mains])
        side = _chain([proj_steps(2, n, lambda i, c: _augment_v(c), vout[n])
                       for n in range(nb)])
        for i, _ in enumerate(main):
            if i + 1 >= voff and i % every == every - 1:
                next(side, None)
        for _ in side:
            pass
        flush(dsts[1])
        extra(len(pace) - n0 - skip)
        flush()
        kv_update([jnp.concatenate([vout[n][2 * r + hi] for hi in range(2)
                                    for n in range(nb)], axis=1)
                   for r in range(2)], last)
        if late is not None:
            late(len(pace) - n0)

    for k in range(len(srcs)):
        cp(k).start()
    zero_s[0] = jnp.uint32(0)
    kvacc[...] = jnp.zeros(kvacc.shape, F32)
    rel = (lax.broadcasted_iota(jnp.int32, (H, D), 1)
           - DH * lax.broadcasted_iota(jnp.int32, (H, D), 0))
    e2 = jnp.where(
        lax.broadcasted_iota(jnp.int32, (VR, DH), 0) >> 1
        == lax.broadcasted_iota(jnp.int32, (VR, DH), 1), 1.0, 0.0).astype(BF16)
    lane8 = lax.broadcasted_iota(jnp.int32, (8, 128), 1)
    sub8 = lax.broadcasted_iota(jnp.int32, (8, 128), 0)
    cp(0).wait()
    m = None
    for d in range(DH):
        sel = jnp.where(rel == d, 1.0, 0.0).astype(BF16)
        t = _dot(wphi_v[d], sel)
        m = t if m is None else m + t
    m2 = _dot(e2, m.astype(BF16))[0:GR]
    relp = lane8 - DH * (sub8 & 1)
    bdts = []
    for kt in range(5):
        r0, r1 = wins[kt]
        pat = m2[:, 128 * kt:128 * (kt + 1)].reshape(5, 8, 128)
        rows = []
        r = r0
        while r < r1:
            g, o = divmod(r, GR)
            n = min(GR - o, r1 - r)
            c0 = GR * g - 128 * kt
            msk = jnp.logical_and(relp >= c0, relp < c0 + DH)
            rows.append(jnp.where(msk[None], pat[o // 8:(o + n) // 8], 0.0))
            r += n
        bdts.append(jnp.concatenate(rows, axis=0)
                    .reshape(r1 - r0, 128).astype(BF16))

    cp(1).wait()
    parts = [fold_part(kt, bdts, wk_v) for kt in range(KF)]
    fold_store(0, parts, range(KF))
    cp(2).wait()
    cp(3).wait()
    for i in range(HB // PG):
        lo, hi = ln_pair(i, 2 * PG * i)
        xn0[_hs(PG * i, PG * (i + 1)), :] = _pk(lo)
        xn0[_hs(HB + PG * i, HB + PG * (i + 1)), :] = _pk(hi)
    parts += [fold_part(kt, bdts, wk_v) for kt in range(KF, 5)]
    fold_store(0, parts, range(KF, 5))
    for r in range(2):
        phi = _feature_map(note(_dot_nt(
            _upk(wT[_hs(DHALF * r, DHALF * (r + 1)), :]), _upk(xn0[...]))))
        for hi in range(2):
            phik[_hs(D * r, D * (r + 1)), TH * hi:TH * hi + HB] = _pk(
                phi[:, HB * hi:HB * (hi + 1)])
    w_sums(0, 2)
    cp(4).wait()
    cp(5).wait()
    for i in range(HB // PG, TH // PG):
        ln_pair(i, 2 * PG * i)
    fold_store(D, [fold_part(kt, bdts, wq_v) for kt in range(5)], range(5))
    for _ in proj_steps(0, 1, store_phi(phik, 1), [None] * 4):
        pass
    flush()
    w_sums(1, 7)
    cp(6).wait()
    cp(7).wait()
    wT[_hs(2 * D, 3 * D), :] = _pk(wv_v[...].T)
    w_sums(2, 0)
    p1_run(0, ((1, 0), (1, 1)), 8, 1, 10, lambda n: ln_next(1, n), False)
    cp(8).wait()
    cp(9).wait()

    all_mains = ((0, 0), (0, 1), (1, 0), (1, 1))

    def p1_body(t, carry):
        @pl.when(t == 2)
        def _():
            cp(10).wait()

        p1_run(t, all_mains, 12, 2, 0, lambda n: ln_next(t + 1, n), False,
               lambda n: run_jobs(
                   ffn_sums_jobs(wgu_v.at[t - 1], sgu.at[t - 1], True)[NSH:], n))
        return carry

    lax.fori_loop(1, NT - 1, p1_body, 0)
    cp(11).wait()
    cp(12).wait()

    p1_run(NT - 1, all_mains, 12, 2, 0,
           lambda n: block_sums([(wo_v, so, 0, KH, KH)], _rhs_sums, n), True,
           lambda n: run_jobs(
               ffn_sums_jobs(wgu_v.at[0], sgu.at[0], True)[:NSH]
               + ffn_sums_jobs(wgu_v.at[1], sgu.at[1], True)[:NSH]
               + ffn_sums_jobs(wd_v, sd, False), n))

    def att_num(ti, b):
        def phi(g):
            rows = _hs(PR * g, PR * (g + 1))
            return _upk(jnp.concatenate(
                [phiq[ti, rows, c0:c0 + HB] for c0 in (HB * b, TH + HB * b)],
                axis=1))

        gnum = [None] * NG
        for g in GORD:
            gnum[g] = _dot(_upk(kvb[g]), phi(g))
        sub = lax.broadcasted_iota(jnp.int32, (8, 2 * HB), 0) < 4
        pieces = []
        for g in range(NG):
            rec = _recip(gnum[g][GR:VR] + DEN_EPS)
            rot = pltpu.roll(rec, 4, 0)
            ra = jnp.where(sub, rec, rot)
            rb = jnp.where(sub, rot, rec)
            scale = jnp.concatenate([ra, ra, rec, rb, rb], axis=0)
            pieces.append(gnum[g][0:GR] * scale)
        return jnp.concatenate(pieces, axis=0)

    def zero_of(tile):
        if tile is None:
            return None
        return pltpu.bitcast(pltpu.bitcast(tile, U32) & zero_s[0], F32)

    def att_sums(ot, z):
        sums = _lhs_sums(_add_tile(ot[0:KH, :HB], z), ot[KH:2 * KH, :HB],
                         ot[0:KH, HB:], _add_tile(ot[KH:2 * KH, HB:], z))
        st = jnp.concatenate(
            [jnp.concatenate([v[:128], v[128:]], axis=1) for v in sums], axis=0)
        st = st.astype(BF16).T
        return [jnp.concatenate([st[:HB, 128 * j:128 * (j + 1)],
                                 st[HB:, 128 * j:128 * (j + 1)]], axis=1)
                for j in range(5)]

    def att_out(ti, b, ot, tile):
        xt, xb = _split_rows(x_rows(ti * T + 2 * HB * b, 2 * HB))
        o = ot.astype(BF16).T
        c5 = _dot(o, wo_v[:, 2 * KH:D])
        r5 = _dot(o[:, 2 * KH:], wo_v[2 * KH:D, 0:2 * KH])
        sums = att_sums(ot, zero_of(tile))
        lhs = _lhs_ops(sums, o[:HB, 0:KH], o[HB:, KH:2 * KH])
        rhs = _rhs_ops([_upk(so[j]) for j in range(5)],
                       wo_v[0:KH, 0:KH], wo_v[KH:2 * KH, KH:2 * KH])
        mm = lambda i: _dot(lhs[i], rhs[i])
        m2, m3, m4, m0 = mm(2), mm(3), mm(4), mm(0)
        c12 = m2 + m4 + r5[:HB, KH:]
        c11 = m3 - m4 + m0 + mm(6) + r5[:HB, :KH]
        ht = xt + jnp.concatenate([c11, c12, c5[:HB]], axis=1)
        m1 = mm(1)
        c21 = m3 + m1 + r5[HB:, :KH]
        c22 = m2 - m1 + m0 + mm(5) + r5[HB:, KH:]
        hb = xb + jnp.concatenate([c21, c22, c5[HB:]], axis=1)
        return (ht, hb), [c5, r5, m2, m3, m4, m0, m1]

    def out_cp(r0, n):
        rows = pl.ds(pl.multiple_of(r0, 16), n)
        return pltpu.make_async_copy(o_v.at[rows], o_hbm.at[rows], sems.at[0])

    class Ffn:
        def __init__(self, base, halves, tq, tiles=None):
            ht, hb = halves
            zs = [None, None]
            if tiles is not None:
                n = HB // LNR
                pick = [zero_of(tiles[k * len(tiles) // n][0:8, :]) for k in range(n)]
                zs = [jnp.concatenate([z for z in pick for _ in range(LNR // 8)],
                                      axis=0)] * 2
            nt_, nb = _layernorm_shifted(ht, zs[0]), _layernorm_shifted(hb, zs[1])
            self.log = []
            self.base, self.tq = base, tq
            self.hn = (nt_[:, 0:KH], nt_[:, KH:2 * KH], nb[:, 0:KH], nb[:, KH:2 * KH])
            self.lhs = {}
            self.a5 = [nt_[:, 2 * KH:].astype(BF16), nb[:, 2 * KH:].astype(BF16)]
            self.cs = [ht[:, 0:KH], ht[:, KH:2 * KH], hb[:, 0:KH], hb[:, KH:2 * KH]]
            self.c5 = jnp.concatenate([ht[:, 2 * KH:], hb[:, 2 * KH:]], axis=0)
            self.act = {}

        def up(self, p):
            cols = (slice(NW * p, NW * (p + 1)), slice(FH + NW * p, FH + NW * (p + 1)))

            def proj(m):
                rest = [functools.partial(_dot, a, wgu_v[m, 2 * KH:D, c])
                        for a in self.a5 for c in cols]

                def lhs_row(i, tile):
                    if i not in self.lhs:
                        self.lhs[i] = [v.astype(BF16) for v in
                                       _lhs_row(self.hn, i, zero_of(tile))]
                    return self.lhs[i]

                return _strassen2(
                    lhs_row,
                    lambda i, j: _upk(sgu[m, 7 * i + j, :, 128 * p:128 * (p + 1)]),
                    rest, log=self.log)

            g, u = proj(0), proj(1)
            self.act[p] = [_gelu(g[i]) * u[i] for i in range(4)]

        def down(self, p):
            act = self.act.pop(p)

            def last_tile(k):
                a = jnp.concatenate([act[k], act[2 + k]], axis=0).astype(BF16)
                r0 = FH * k + NW * p
                self.c5 = self.c5 + _dot(a, wd_v[r0:r0 + NW, 2 * KH:D])

            last_tile(0)
            rhs = lambda i, j: _upk(sd[7 * i + j, _hs(128 * p, 128 * (p + 1)), 0:128])

            def mult(a, cs, mid, plag):
                def swap(b):
                    if SWAP[p] & 1:
                        b = [b[2], b[3], b[0], b[1]]
                    if SWAP[p] & 2:
                        h = b[0].shape[0] // 2
                        b = [jnp.concatenate([v[h:], v[:h]], axis=0) for v in b]
                    return b

                a = swap(a)
                order = ((2, 3, 1, None, 0, 5, 4, 6) if SWAP[p] & 1
                         else (2, 4, 5, None, 3, 1, 0, 6))
                return swap(_strassen2(
                    lambda i, tile: [v.astype(BF16) for v in
                                     _lhs_row(a, i, zero_of(tile))],
                    rhs, swap(cs), order, mid, plag))

            if p < FH // NW - 1:
                self.cs = mult(act, self.cs, lambda: last_tile(1), 3)
                return
            tq, hq = self.tq, HB // 2
            for q in range(0, hq, tq):
                pick = lambda c: jnp.concatenate(
                    [c[q:q + tq], c[hq + q:hq + q + tq]], axis=0)
                f = mult([pick(a) for a in act], [pick(c) for c in self.cs],
                         lambda: last_tile(1) if q == 0 else None, 3 * hq // tq)
                top = jnp.concatenate([f[0], f[1], pick(self.c5[:HB])], axis=1)
                bot = jnp.concatenate([f[2], f[3], pick(self.c5[HB:])], axis=1)
                for k in range(2):
                    res = _merge_rows(top[tq * k:tq * (k + 1)], bot[tq * k:tq * (k + 1)])
                    r0 = self.base + 2 * (hq * k + q)
                    o_v[pl.ds(pl.multiple_of(r0, 2 * tq), 2 * tq), :] = res.astype(BF16)
                    out_cp(r0, 2 * tq).start()

    def p2_body(t, carry):
        nb = TH // HB
        ots = [att_num(t, b) for b in range(nb)]
        hs = []
        tile = ots[1][SA:SA + 8, 0:128]
        for b in range(nb):
            h, res = att_out(t, b, ots[b], tile)
            hs.append(h)
            tile = res[SB][0:8, 0:128]
        tiles = None
        for b in range(nb):
            f = Ffn(t * T + 2 * HB * b, hs[b], TQ if b + 1 == nb else HB // 2, tiles)
            for p in range(FH // NW):
                f.up(p)
                f.down(p)
            tiles = f.log[LN0:LN1]
        return carry

    lax.fori_loop(0, NT, p2_body, 0)
    pltpu.make_async_copy(o_v, o_hbm, sems.at[0]).wait()


@jax.jit
def pallas_sequential_preLN__linear_kernel_hedgehog__geglu_ffn__prompt_kernel(
    A_x: jax.Array,
    A_wqkv: jax.Array,
    A_w_phi: jax.Array,
    A_wo: jax.Array,
    B_x: jax.Array,
    B_w_gate: jax.Array,
    B_w_up: jax.Array,
    B_w_down: jax.Array,
):
    del B_x
    x = A_x.reshape(S, D)
    wphi = jnp.transpose(A_w_phi, (1, 2, 0))
    any_spec = pl.BlockSpec(memory_space=pl.ANY)
    out = pl.pallas_call(
        _kernel,
        in_specs=[any_spec] * 7,
        out_specs=any_spec,
        out_shape=jax.ShapeDtypeStruct((S, D), BF16),
        scratch_shapes=[
            pltpu.VMEM((S, D), BF16),
            pltpu.VMEM((DH, DH, H), BF16),
            pltpu.VMEM((D, D), BF16),
            pltpu.VMEM((D, D), BF16),
            pltpu.VMEM((D, D), BF16),
            pltpu.VMEM((D, D), BF16),
            pltpu.VMEM((2, D, F), BF16),
            pltpu.VMEM((F, D), BF16),
            pltpu.VMEM((3 * D // 2, D), U32),
            pltpu.VMEM((3, 5, DHALF // 2, KH), U32),
            pltpu.VMEM((HB, D), U32),
            pltpu.VMEM((7, TH // 2, KH), U32),
            pltpu.VMEM((TH // 2, 256), U32),
            pltpu.VMEM((NT, D, T), U32),
            pltpu.VMEM((D, T), U32),
            pltpu.VMEM((NG, VR, PR), F32),
            pltpu.VMEM((NG, VR // 2, PR), U32),
            pltpu.VMEM((2, 49, KH // 4, FH // 2), U32),
            pltpu.VMEM((49, FH // 4, KH), U32),
            pltpu.VMEM((5, KH // 2, KH), U32),
            pltpu.VMEM((S, D), BF16),
            pltpu.SMEM((1,), U32),
            pltpu.SemaphoreType.DMA((8,)),
        ],
        compiler_params=pltpu.CompilerParams(
            vmem_limit_bytes=100 * 1024 * 1024),
        name="hedgehog_block",
    )(x, A_wqkv, wphi, A_wo, B_w_gate, B_w_up, B_w_down)
    return out.reshape(1, S, D)
```
